```python
import jax
import jax.numpy as jnp

def _softmax(x, axis=-1):
    return jax.nn.softmax(x, axis=axis)

def _gelu(x):
    return jax.nn.gelu(x, approximate=True)

def _silu(x):
    return jax.nn.silu(x)

def _sigmoid(x):
    return jax.nn.sigmoid(x)

def _layernorm(x, axis=-1, eps=1e-05):
    m = jnp.mean(x, axis=axis, keepdims=True)
    v = jnp.var(x, axis=axis, keepdims=True)
    return (x - m) / jnp.sqrt(v + eps)

def _scatter_add(tgt, idx, src, axis=0):
    return tgt.at[idx].add(src)

def _segment_sum(src, seg, n):
    return jax.ops.segment_sum(src, seg, n)

class _Rng:

    def __init__(self, key):
        self._k = key

    def _next(self):
        self._k, sub = jax.random.split(self._k)
        return sub

    def normal(self, shape):
        return jax.random.normal(self._next(), shape, dtype=jnp.bfloat16)

    def randint(self, lo, hi, shape):
        return jax.random.randint(self._next(), shape, lo, hi, dtype=jnp.int32)

    def uniform(self, shape, lo=0.0, hi=1.0):
        return jax.random.uniform(self._next(), shape, jnp.bfloat16, lo, hi)

    def permutation(self, n):
        return jax.random.permutation(self._next(), n)
kernel_name = 'standalone__autoregressive_conv_wavernn__speech'

def setup_inputs():
    _rng = _Rng(jax.random.key(int.from_bytes(__import__("os").urandom(4), "little")))
    _w = lambda a: (lambda t: t.astype(jnp.bfloat16) if jnp.issubdtype(t.dtype, jnp.floating) else t)(jnp.asarray(a))
    B, T, D, K = (2, 16000, 256, 31)
    return {'x': _w((lambda *s: _rng.normal(s) * 0.05)(B, T, D)), 'w': _w((lambda *s: _rng.normal(s) * 0.05)(K, D, 2 * D))}

def reference(x, w):
    B, T, D = x.shape
    K = w.shape[0]
    dil = 2
    pad = (K - 1) * dil
    xp = jnp.pad(x, ((0, 0), (pad, 0), (0, 0)))
    h = jnp.einsum('btd,de->bte', xp[:, 0:T, :], w[0])
    for i in range(1, K):
        h = h + jnp.einsum('btd,de->bte', xp[:, i * dil:i * dil + T, :], w[i])
    f, g = (h[..., :D].copy(), h[..., D:].copy())
    return jnp.tanh(f) * _sigmoid(g)
```

```python
import functools
import numpy as np
import jax, jax.numpy as jnp
from jax import lax
from jax.experimental import pallas as pl
from jax.experimental.pallas import tpu as pltpu
import ml_dtypes

N=128; L=96; NK=64
SX=196; SW=196; SI=132; SY=340

def consts(K):
    th = 2*np.pi*(np.arange(NK)+0.5)/N
    n = np.arange(N)
    F = np.concatenate([np.cos(th[:,None]*n[None]), np.sin(th[:,None]*n[None])],0)
    Fp = np.zeros_like(F); Fp[:,0::2]=F[:,:64]; Fp[:,1::2]=F[:,64:]
    i = np.arange(32)
    off = 32-(K-1)
    Gc = np.cos(th[:,None]*(i+off)[None]); Gs=-np.sin(th[:,None]*(i+off)[None])
    Gc[:,K:]=0; Gs[:,K:]=0
    GW = np.zeros((512,128))
    for qs in range(2):
        for kg in range(8):
            base = qs*256+kg*32
            for h,(G,dpar) in enumerate([(Gc,0),(Gc,1),(Gs,0),(Gs,1)]):
                GW[base+h*8:base+h*8+8, 2*(qs*32+i)+dpar] = G[kg*8:kg*8+8,:]
    r = np.arange(L)
    IA = np.zeros((L,128)); IA[:,0::2]=(2/N)*np.cos(r[:,None]*th[None]); IA[:,1::2]=(2/N)*np.sin(r[:,None]*th[None])
    c = lambda a: a.astype(np.float32).astype(ml_dtypes.bfloat16)
    return c(Fp), c(GW), c(IA)

def make(B,T,D,K, UF=2, UI=2, UM=1, phases='WFMI'):
    M = T//2; NJ = -(-M//L); MP = (NJ-1)*L+N; NR = B*NJ
    f32=jnp.float32; bf16=jnp.bfloat16; i32=jnp.int32
    def bc(x,t): return pltpu.bitcast(x,t)
    def pack(a,b): return pltpu.pack_elementwise([a,b], packed_dtype=bf16)
    def kernel(x_hbm, w_hbm, fa_ref, gw_ref, ia_ref, out_hbm,
               xbuf, wbuf, Xf, Wf, Yp, obuf, xsem, wsem, osem):
        xb16 = xbuf.bitcast(bf16); wb16 = wbuf.bitcast(bf16); ob16 = obuf.bitcast(bf16)
        def wcopy(et,i):
            return pltpu.make_async_copy(w_hbm.at[i,:,pl.ds(et*128,128)], wb16.at[et,pl.ds(i*(2*SI),D),:], wsem.at[et])
        def xcopy(b,dt):
            return pltpu.make_async_copy(x_hbm.at[b,:,pl.ds(dt*128,128)], xb16.at[b*2+dt,pl.ds(64,T),:], xsem.at[b*2+dt])
        def ocopy(b,c):
            return pltpu.make_async_copy(ob16.at[b,pl.ds(0,T),:], out_hbm.at[b,:,pl.ds(c*128,128)], osem.at[b])
        ets = lambda c: (c, D//128+c)
        for et in ets(0):
            @pl.loop(0,K)
            def _(i): wcopy(et,i).start()
        for b in range(B):
            for dt in range(2): xcopy(b,dt).start()
        for et in ets(1):
            @pl.loop(0,K)
            def _(i): wcopy(et,i).start()
        zero = jnp.zeros
        for s in range(B*2):
            xbuf[s,pl.ds(0,32),:] = zero((32,128),i32)
            xbuf[s,pl.ds(32+M,MP-32-M),:] = zero((MP-32-M,128),i32)
        for et in range(4):
            wbuf[et,pl.ds(K*SI,(32-K)*SI),:] = zero(((32-K)*SI,128),i32)

        def phaseW(c):
            for et in ets(c):
                @pl.loop(0,K)
                def _(i): wcopy(et,i).wait()
            @pl.loop(0,32)
            def _(g):
                tiles=[]
                for qp in range(2):
                    for et in ets(c):
                        q0 = g*4+qp*2
                        t = jnp.concatenate([wbuf[et,pl.ds(q0,32,stride=SI),:], wbuf[et,pl.ds(q0+1,32,stride=SI),:]],axis=0)
                        tiles.append(bc(t,bf16))
                rhs = jnp.concatenate(tiles,axis=1)
                o = jnp.dot(gw_ref[...], rhs, preferred_element_type=f32)
                for qp in range(2):
                    for e2 in range(2):
                        col = (qp*2+e2)*128
                        for qs in range(2):
                            q = g*4+qp*2+qs
                            for kg in range(8):
                                base=qs*256+kg*32
                                r0=o[base:base+8,col:col+128]; r1=o[base+8:base+16,col:col+128]
                                i0=o[base+16:base+24,col:col+128]; i1=o[base+24:base+32,col:col+128]
                                Wf[e2,pl.ds(q*SW+kg*8,8),:] = pack(r0,r1)
                                Wf[e2,pl.ds(q*SW+64+kg*8,8),:] = pack(i0-r0,i1-r1)
                                Wf[e2,pl.ds(q*SW+128+kg*8,8),:] = pack(r0+i0,r1+i1)

        def fblock(b,j):
            tiles=[]
            for dt in range(2):
                X = xbuf[b*2+dt,pl.ds(j*L,N),:]
                top=X[0:64]; bot=X[64:128]
                E = (top & 0xFFFF) | (bot<<16)
                O = lax.shift_right_logical(top,16) | (bot & jnp.int32(-65536))
                tiles += [bc(E,bf16), bc(O,bf16)]
            Y = jnp.dot(fa_ref[...], jnp.concatenate(tiles,axis=1), preferred_element_type=f32)
            J = b*NJ+j
            for dt in range(2):
                Ye=Y[:,dt*256:dt*256+128]; Yo=Y[:,dt*256+128:dt*256+256]
                Xf[dt,pl.ds(J*SX,64),:] = pack(Ye[:64]+Ye[64:], Yo[:64]+Yo[64:])
                Xf[dt,pl.ds(J*SX+64,64),:] = pack(Ye[:64],Yo[:64])
                Xf[dt,pl.ds(J*SX+128,64),:] = pack(Ye[64:],Yo[64:])
        def phaseF():
            for b in range(B):
                xcopy(b,0).wait(); xcopy(b,1).wait()
                @pl.loop(0,NJ//UF)
                def _(jj):
                    for u in range(UF): fblock(b,jj*UF+u)

        NJ2 = NR
        def mbin(k):
            def lhs(v): return jnp.concatenate([bc(Xf[dt,pl.ds(v*64+k,NJ2,stride=SX),:],bf16) for dt in range(2)],axis=1)
            def rhs(v): return jnp.concatenate([bc(Wf[e2,pl.ds(v*64+k,128,stride=SW),:],bf16) for e2 in range(2)],axis=1)
            k1=jnp.dot(lhs(0),rhs(0),preferred_element_type=f32)
            k2=jnp.dot(lhs(1),rhs(1),preferred_element_type=f32)
            k3=jnp.dot(lhs(2),rhs(2),preferred_element_type=f32)
            Yr=k1-k3; Yi=k1+k2
            for e2 in range(2):
                Yp[e2,pl.ds(k*SY,2*NR),:] = pack(Yr[:,e2*128:e2*128+128],Yi[:,e2*128:e2*128+128])
        def phaseM():
            @pl.loop(0,NK//UM)
            def _(kk):
                for u in range(UM): mbin(kk*UM+u)

        def iblock(b,j):
            J=b*NJ+j
            tiles=[]
            for p in range(2):
                for e2 in range(2):
                    tiles.append(bc(Yp[e2,pl.ds(2*J+p,64,stride=SY),:],bf16))
            h = jnp.dot(ia_ref[...], jnp.concatenate(tiles,axis=1), preferred_element_type=f32)
            oe = jnp.tanh(h[:,0:128])*jax.nn.sigmoid(h[:,128:256])
            oo = jnp.tanh(h[:,256:384])*jax.nn.sigmoid(h[:,384:512])
            obuf[b,pl.ds(j*L,L),:] = pack(oe,oo)
        def phaseI(c):
            for b in range(B):
                if c>0: ocopy(b,c-1).wait()
                @pl.loop(0,NJ//UI)
                def _(jj):
                    for u in range(UI): iblock(b,jj*UI+u)
                ocopy(b,c).start()

        with jax.named_scope('W0'): phaseW(0)
        with jax.named_scope('F'): phaseF()
        with jax.named_scope('M0'): phaseM()
        with jax.named_scope('I0'): phaseI(0)
        with jax.named_scope('W1'): phaseW(1)
        with jax.named_scope('M1'): phaseM()
        with jax.named_scope('I1'): phaseI(1)
        for b in range(B): ocopy(b,1).wait()

    fa,gw,ia = consts(K)
    def f(x,w):
        return pl.pallas_call(kernel,
            out_shape=jax.ShapeDtypeStruct((B,T,D),bf16),
            in_specs=[pl.BlockSpec(memory_space=pl.ANY),pl.BlockSpec(memory_space=pl.ANY),
                      pl.BlockSpec(memory_space=pltpu.VMEM),pl.BlockSpec(memory_space=pltpu.VMEM),pl.BlockSpec(memory_space=pltpu.VMEM)],
            out_specs=pl.BlockSpec(memory_space=pl.ANY),
            scratch_shapes=[pltpu.VMEM((B*2,MP,128),i32), pltpu.VMEM((4,32*SI,128),i32),
                            pltpu.VMEM((2,NR*SX,128),i32), pltpu.VMEM((2,128*SW,128),i32),
                            pltpu.VMEM((2,NK*SY,128),i32), pltpu.VMEM((B,NJ*L,128),i32),
                            pltpu.SemaphoreType.DMA((B*2,)), pltpu.SemaphoreType.DMA((4,)), pltpu.SemaphoreType.DMA((B,))],
            compiler_params=pltpu.CompilerParams(vmem_limit_bytes=127*1024*1024),
        )(x,w,jnp.asarray(fa),jnp.asarray(gw),jnp.asarray(ia))
    return f


_CFG = dict(UF=2, UI=2, UM=1)


@jax.jit
def pallas_standalone__autoregressive_conv_wavernn__speech_kernel(x: jax.Array, w: jax.Array):
    B, T, D = x.shape
    K = w.shape[0]
    return make(B, T, D, K, **_CFG)(x, w)
```

```python
import numpy as np
import jax, jax.numpy as jnp
from jax import lax
from jax.experimental import pallas as pl
from jax.experimental.pallas import tpu as pltpu
import ml_dtypes

N=128; L=96; NK=64
SX=196; SW=196; SI=132; SY=340

def _pack_rows(a):
    u = a.astype(np.float32).astype(ml_dtypes.bfloat16).view(np.uint16).astype(np.uint32)
    return (u[0::2] | (u[1::2] << 16)).view(np.int32)

def consts(K):
    th = 2*np.pi*(np.arange(NK)+0.5)/N
    n = np.arange(N)
    F = np.concatenate([np.cos(th[:,None]*n[None]), np.sin(th[:,None]*n[None])],0)
    Fp = np.zeros_like(F); Fp[:,0::2]=F[:,:64]; Fp[:,1::2]=F[:,64:]
    i = np.arange(32)
    off = 32-(K-1)
    Gc = np.cos(th[:,None]*(i+off)[None]); Gs=-np.sin(th[:,None]*(i+off)[None])
    Gc[:,K:]=0; Gs[:,K:]=0
    GW = np.zeros((512,128))
    for qs in range(2):
        for kg in range(8):
            base = qs*256+kg*32
            for h,(G,dpar) in enumerate([(Gc,0),(Gc,1),(Gs,0),(Gs,1)]):
                GW[base+h*8:base+h*8+8, 2*(qs*32+i)+dpar] = G[kg*8:kg*8+8,:]
    r = np.arange(L)
    IA = np.zeros((L,128)); IA[:,0::2]=(2/N)*np.cos(r[:,None]*th[None]); IA[:,1::2]=(2/N)*np.sin(r[:,None]*th[None])
    return np.concatenate([_pack_rows(GW),_pack_rows(Fp),_pack_rows(IA)],0)

def make(B,T,D,K, UF=21, UI=21, UM=8, UW=4, sched=None, scopes=True):
    M = T//2; NJ = -(-M//L); MP = (NJ-1)*L+N; NR = B*NJ
    f32=jnp.float32; bf16=jnp.bfloat16; i32=jnp.int32
    NP=4; JP=NJ//NP; TP=JP*2*L
    TL=T-(NP-1)*TP
    assert NJ%NP==0 and JP%UF==0 and JP%UI==0 and 16%UW==0 and NK%UM==0
    WI=32//UW
    def bc(x,t): return pltpu.bitcast(x,t)
    def pack(a,b): return pltpu.pack_elementwise([a,b], packed_dtype=bf16)
    import contextlib
    scope = jax.named_scope if scopes else (lambda n: contextlib.nullcontext())
    def kernel(x_hbm, w_hbm, c_hbm, out_hbm,
               cbuf, xbuf, wbuf, Xf, Wf, Yp, obuf, csem, xsem, wsem, osem):
        xb16 = xbuf.bitcast(bf16); wb16 = wbuf.bitcast(bf16); ob16 = obuf.bitcast(bf16)
        mk=pltpu.make_async_copy
        ccopy = mk(c_hbm, cbuf, csem.at[0])
        def wcopy(et,i):
            return mk(w_hbm.at[i,:,pl.ds(pl.multiple_of(et*128,128),128)], wb16.at[et,pl.ds(pl.multiple_of(i*(2*SI),8),D),:], wsem.at[et])
        def startW(et):
            @pl.loop(0,K)
            def _(i): wcopy(et,i).start()
        def waitW(et):
            @pl.loop(0,K)
            def _(i): wcopy(et,i).wait()
        def xcopy(b,dt,p,n):
            t0=pl.multiple_of(p*TP,8)
            return mk(x_hbm.at[b,pl.ds(t0,n),pl.ds(dt*128,128)], xb16.at[b*2+dt,pl.ds(64+t0,n),:], xsem.at[b*2+dt,p])
        def xstart(g):
            b,p=divmod(g,NP)
            for dt in range(2): xcopy(b,dt,p,TP if p<NP-1 else TL).start()
        def xwait(b,p):
            @pl.when(p<NP-1)
            def _():
                for dt in range(2): xcopy(b,dt,p,TP).wait()
            @pl.when(p==NP-1)
            def _():
                for dt in range(2): xcopy(b,dt,p,TL).wait()
        def ocopy(b,c,p,n):
            t0=pl.multiple_of(p*TP,8)
            return mk(ob16.at[b,pl.ds(t0,n),:], out_hbm.at[b,pl.ds(t0,n),pl.ds(pl.multiple_of(c*128,128),128)], osem.at[b,p])
        def ostart(b,c,p):
            @pl.when(p<NP-1)
            def _(): ocopy(b,c,p,TP).start()
            @pl.when(p==NP-1)
            def _(): ocopy(b,c,p,TL).start()
        def owait(b,c,p):
            @pl.when(p<NP-1)
            def _(): ocopy(b,c,p,TP).wait()
            @pl.when(p==NP-1)
            def _(): ocopy(b,c,p,TL).wait()

        ccopy.start()
        startW(0)
        zero = jnp.zeros
        for s in range(B*2):
            xbuf[s,pl.ds(0,32),:] = zero((32,128),i32)
            xbuf[s,pl.ds(32+M,MP-32-M),:] = zero((MP-32-M,128),i32)
        for et in range(4):
            wbuf[et,pl.ds(K*SI,(32-K)*SI),:] = zero(((32-K)*SI,128),i32)
        ccopy.wait()
        GWr = lambda: bc(cbuf[0:256,:],bf16)
        FAr = lambda: bc(cbuf[256:320,:],bf16)
        IAr = lambda: bc(cbuf[320:368,:],bf16)

        def wgroup(et,e2,g):
            tiles=[]
            for qp in range(4):
                q0 = g*8+qp*2
                t = jnp.concatenate([wbuf[et,pl.ds(q0,32,stride=SI),:], wbuf[et,pl.ds(q0+1,32,stride=SI),:]],axis=0)
                tiles.append(bc(t,bf16))
            o = jnp.dot(GWr(), jnp.concatenate(tiles,axis=1), preferred_element_type=f32)
            for qp in range(4):
                col = qp*128
                for qs in range(2):
                    q = g*8+qp*2+qs
                    for kg in range(8):
                        base=qs*256+kg*32
                        r0=o[base:base+8,col:col+128]; r1=o[base+8:base+16,col:col+128]
                        i0=o[base+16:base+24,col:col+128]; i1=o[base+24:base+32,col:col+128]
                        Wf[e2,pl.ds(q*SW+kg*8,8),:] = pack(r0,r1)
                        Wf[e2,pl.ds(q*SW+64+kg*8,8),:] = pack(i0-r0,i1-r1)
                        Wf[e2,pl.ds(q*SW+128+kg*8,8),:] = pack(r0+i0,r1+i1)
        wsched = sched or {0:[0],3:[1],5:[2],7:[3]}
        def phaseW(c):
            @pl.loop(0,WI)
            def _(it):
                e2 = it//(WI//2); et = c+2*e2
                @pl.when(it%(WI//2)==0)
                def _(): waitW(et)
                @pl.when(c==0)
                def _():
                    @pl.when(it==0)
                    def _(): startW(2)
                    for i0,ps in wsched.items():
                        @pl.when(it==i0*WI//8)
                        def _():
                            for g in ps: xstart(g)
                gb=(it%(WI//2))*UW
                for u in range(UW): wgroup(et,e2,gb+u)

        def fblock(b,j):
            tiles=[]
            for dt in range(2):
                X = xbuf[b*2+dt,pl.ds(j*L,N),:]
                top=X[0:64]; bot=X[64:128]
                E = (top & 0xFFFF) | (bot<<16)
                O = lax.shift_right_logical(top,16) | (bot & jnp.int32(-65536))
                tiles += [bc(E,bf16), bc(O,bf16)]
            Y = jnp.dot(FAr(), jnp.concatenate(tiles,axis=1), preferred_element_type=f32)
            J = b*NJ+j
            for dt in range(2):
                Ye=Y[:,dt*256:dt*256+128]; Yo=Y[:,dt*256+128:dt*256+256]
                Xf[dt,pl.ds(J*SX,64),:] = pack(Ye[:64]+Ye[64:], Yo[:64]+Yo[64:])
                Xf[dt,pl.ds(J*SX+64,64),:] = pack(Ye[:64],Yo[:64])
                Xf[dt,pl.ds(J*SX+128,64),:] = pack(Ye[64:],Yo[64:])
        FI=JP//UF
        nw=len(sum(wsched.values(),[]))
        def phaseF():
            @pl.loop(0,B*NP*FI)
            def _(it):
                g=it//FI; b=g//NP; p=g%NP
                @pl.when(it%FI==0)
                def _():
                    for g0 in range(B*NP):
                        if g0+nw<B*NP:
                            @pl.when(g==g0)
                            def _(): xstart(g0+nw)
                    @pl.when(g==B*NP-2)
                    def _(): startW(1)
                    @pl.when(g==B*NP-1)
                    def _(): startW(3)
                    xwait(b,p)
                j0=p*JP+(it%FI)*UF
                for u in range(UF): fblock(b,j0+u)

        def mbin(k):
            def lhs(v): return jnp.concatenate([bc(Xf[dt,pl.ds(v*64+k,NR,stride=SX),:],bf16) for dt in range(2)],axis=1)
            def rhs(v): return jnp.concatenate([bc(Wf[e2,pl.ds(v*64+k,128,stride=SW),:],bf16) for e2 in range(2)],axis=1)
            k1=jnp.dot(lhs(0),rhs(0),preferred_element_type=f32)
            k2=jnp.dot(lhs(1),rhs(1),preferred_element_type=f32)
            k3=jnp.dot(lhs(2),rhs(2),preferred_element_type=f32)
            Yr=k1-k3; Yi=k1+k2
            for e2 in range(2):
                Yp[e2,pl.ds(k*SY,2*NR),:] = pack(Yr[:,e2*128:e2*128+128],Yi[:,e2*128:e2*128+128])
        def phaseM():
            @pl.loop(0,NK//UM)
            def _(kk):
                for u in range(UM): mbin(kk*UM+u)

        def iblock(b,j):
            J=b*NJ+j
            tiles=[]
            for p in range(2):
                for e2 in range(2):
                    tiles.append(bc(Yp[e2,pl.ds(2*J+p,64,stride=SY),:],bf16))
            h = jnp.dot(IAr(), jnp.concatenate(tiles,axis=1), preferred_element_type=f32)
            oe = jnp.tanh(h[:,0:128])*(jnp.tanh(h[:,128:256]*0.5)*0.5+0.5)
            oo = jnp.tanh(h[:,256:384])*(jnp.tanh(h[:,384:512]*0.5)*0.5+0.5)
            obuf[b,pl.ds(j*L,L),:] = pack(oe,oo)
        II=JP//UI
        def phaseI(c):
            @pl.loop(0,B*NP*II)
            def _(it):
                g=it//II; b=g//NP; p=g%NP
                @pl.when(jnp.logical_and(c>0, it%II==0))
                def _(): owait(b,c-1,p)
                j0=p*JP+(it%II)*UI
                for u in range(UI): iblock(b,j0+u)
                @pl.when(it%II==II-1)
                def _(): ostart(b,c,p)

        @pl.loop(0,2)
        def _(c):
            with scope('W'): phaseW(c)
            @pl.when(c==0)
            def _():
                with scope('F'): phaseF()
            with scope('M'): phaseM()
            with scope('I'): phaseI(c)
        with scope('end'):
            for b in range(B):
                for p in range(NP): ocopy(b,1,p,TP if p<NP-1 else TL).wait()

    cst = consts(K)
    def f(x,w):
        return pl.pallas_call(kernel,
            out_shape=jax.ShapeDtypeStruct((B,T,D),bf16),
            in_specs=[pl.BlockSpec(memory_space=pl.ANY)]*3,
            out_specs=pl.BlockSpec(memory_space=pl.ANY),
            scratch_shapes=[pltpu.VMEM(cst.shape,i32),pltpu.VMEM((B*2,MP,128),i32), pltpu.VMEM((4,32*SI,128),i32),
                            pltpu.VMEM((2,NR*SX,128),i32), pltpu.VMEM((2,128*SW,128),i32),
                            pltpu.VMEM((2,NK*SY,128),i32), pltpu.VMEM((B,NJ*L,128),i32),
                            pltpu.SemaphoreType.DMA((1,)),
                            pltpu.SemaphoreType.DMA((B*2,NP)), pltpu.SemaphoreType.DMA((4,)), pltpu.SemaphoreType.DMA((B,NP))],
            compiler_params=pltpu.CompilerParams(vmem_limit_bytes=127*1024*1024),
        )(x,w,jnp.asarray(cst))
    return f


@jax.jit
def pallas_standalone__autoregressive_conv_wavernn__speech_kernel(x: jax.Array, w: jax.Array):
    B, T, D = x.shape
    K = w.shape[0]
    return make(B, T, D, K, scopes=False)(x, w)
```

```python
import contextlib
import numpy as np
import jax, jax.numpy as jnp
from jax import lax
from jax.experimental import pallas as pl
from jax.experimental.pallas import tpu as pltpu
import ml_dtypes

N=128; L=96; NK=64
SX=196; SW=196; SI=132; SY=340

def _pack_rows(a):
    u = a.astype(np.float32).astype(ml_dtypes.bfloat16).view(np.uint16).astype(np.uint32)
    return (u[0::2] | (u[1::2] << 16)).view(np.int32)

def consts(K):
    th = 2*np.pi*(np.arange(NK)+0.5)/N
    n = np.arange(N)
    off = 32-(K-1)
    F = np.concatenate([np.cos(th[:,None]*(n[None]-off)), np.sin(th[:,None]*(n[None]-off))],0)
    Fp = np.zeros_like(F); Fp[:,0::2]=F[:,:64]; Fp[:,1::2]=F[:,64:]
    i = np.arange(32)
    Gc = np.cos(th[:,None]*i[None]); Gs=-np.sin(th[:,None]*i[None])
    Gc[:,K:]=0; Gs[:,K:]=0
    GW = np.zeros((512,128))
    for qs in range(2):
        for kg in range(8):
            base = qs*256+kg*32
            for h,(G,dpar) in enumerate([(Gc,0),(Gc,1),(Gs,0),(Gs,1)]):
                GW[base+h*8:base+h*8+8, 2*(qs*32+i)+dpar] = G[kg*8:kg*8+8,:]
    r = np.arange(L)
    IA = np.zeros((L,128)); IA[:,0::2]=(2/N)*np.cos(r[:,None]*th[None]); IA[:,1::2]=(2/N)*np.sin(r[:,None]*th[None])
    return np.concatenate([_pack_rows(GW),_pack_rows(Fp),_pack_rows(IA)],0)

def f32c(v): return float(np.float32(v))
def pass1(u):
    out=[None]*8
    for kp in range(4):
        ph = 2*np.pi*(kp+0.5)/16
        c1,s1 = np.cos(ph),-np.sin(ph); c2,s2=np.cos(2*ph),-np.sin(2*ph); c3,s3=np.cos(3*ph),-np.sin(3*ph)
        Er = u[0]+u[2]*f32c(c2); Ei = u[2]*f32c(s2)
        if u[3] is not None:
            Or = u[1]*f32c(c1)+u[3]*f32c(c3); Oi = u[1]*f32c(s1)+u[3]*f32c(s3)
        else:
            Or = u[1]*f32c(c1); Oi = u[1]*f32c(s1)
        out[kp] = (Er+Or, Ei+Oi)
        out[7-kp] = (Er-Or, Oi-Ei)
    return out
def cmul(z,ang):
    c,s=f32c(np.cos(ang)),f32c(np.sin(ang))
    return (z[0]*c - z[1]*s, z[0]*s + z[1]*c)
def dft4(x):
    a=(x[0][0]+x[2][0], x[0][1]+x[2][1]); b=(x[0][0]-x[2][0], x[0][1]-x[2][1])
    c=(x[1][0]+x[3][0], x[1][1]+x[3][1]); d=(x[1][0]-x[3][0], x[1][1]-x[3][1])
    return [(a[0]+c[0],a[1]+c[1]), (b[0]+d[1], b[1]-d[0]), (a[0]-c[0],a[1]-c[1]), (b[0]-d[1], b[1]+d[0])]
def pass2(P,kp):
    th=2*np.pi*(kp+0.5)/N
    Q=[P[0]]+[cmul(P[r],-th*r) for r in range(1,8)]
    A=dft4([Q[0],Q[2],Q[4],Q[6]]); Bv=dft4([Q[1],Q[3],Q[5],Q[7]])
    h=f32c(np.sqrt(0.5))
    B=[Bv[0],
       ((Bv[1][0]+Bv[1][1])*h, (Bv[1][1]-Bv[1][0])*h),
       (Bv[2][1], None),
       ((Bv[3][1]-Bv[3][0])*h, None)]
    res={}
    for s in range(4):
        Ar,Ai=A[s]
        if s==2:   Br,nBi=Bv[2][1],Bv[2][0]
        elif s==3: Br,nBi=B[3][0],(Bv[3][0]+Bv[3][1])*h
        else:      Br,Bi=B[s]; nBi=None
        if nBi is None:
            Re=Ar+Br; Im=Ai+Bi; Re2=Ar-Br; nIm2=Bi-Ai
        else:
            Re=Ar+Br; Im=Ai-nBi; Re2=Ar-Br; nIm2=(0.0 - nBi)-Ai if False else None
            nIm2 = -(nBi+Ai)
        k=kp+16*s
        res[k]=(Re, Im-Re, Re+Im)
        km=127-kp-16*(s+4)
        res[km]=(Re2, nIm2-Re2, Re2+nIm2)
    return res

def p2half(Q,odd):
    def half(x):
        if not odd:
            a=(x[0][0]+x[2][0], x[0][1]+x[2][1]); c=(x[1][0]+x[3][0], x[1][1]+x[3][1])
            return {0:(a[0]+c[0],a[1]+c[1]), 2:(a[0]-c[0],a[1]-c[1])}
        b=(x[0][0]-x[2][0], x[0][1]-x[2][1]); d=(x[1][0]-x[3][0], x[1][1]-x[3][1])
        return {1:(b[0]+d[1], b[1]-d[0]), 3:(b[0]-d[1], b[1]+d[0])}
    A=half([Q[0],Q[2],Q[4],Q[6]]); Bv=half([Q[1],Q[3],Q[5],Q[7]])
    h=f32c(np.sqrt(0.5)); res={}
    for s in A:
        Ar,Ai=A[s]; br,bi=Bv[s]
        if s==0:   Br,Bi,nBi=br,bi,None
        elif s==1: Br,Bi,nBi=(br+bi)*h,(bi-br)*h,None
        elif s==2: Br,Bi,nBi=bi,None,br
        else:      Br,Bi,nBi=(bi-br)*h,None,(br+bi)*h
        Re=Ar+Br; Re2=Ar-Br
        if nBi is None: Im=Ai+Bi; nIm2=Bi-Ai
        else:           Im=Ai-nBi; nIm2=(-1.0*0+0) if False else None
        res[s]=(Re,Im,Re2,Ai,Bi,nBi)
    return res

def make(B,T,D,K, UI=14, UM=8, scopes=True, vpu=True, cmode=0, flags=None, TOK=1, TOKR=(0,1), TOKH=(0,1), P1SPLIT=True, LAG=0, TAIL=8, DORD=(0,1,2,3,4,5)):
    M = T//2; NJ = -(-M//L); MP = (NJ-1)*L+N; NR = B*NJ
    f32=jnp.float32; bf16=jnp.bfloat16; i32=jnp.int32
    NP=4; JP=NJ//NP; TP=JP*2*L; TL=T-(NP-1)*TP
    assert NJ%NP==0 and NJ%UI==0 and NK%UM==0 and UM%2==0
    def bc(x,t): return pltpu.bitcast(x,t)
    def pack(a,b): return pltpu.pack_elementwise([a,b], packed_dtype=bf16)
    scope = jax.named_scope if scopes else (lambda n: contextlib.nullcontext())
    R3=2*192*128
    assert 4*MP<=R3
    R2=2*128*SW
    assert B*NJ*L<=R2
    def kernel(x_hbm, w_hbm, c_hbm, out_hbm,
               cbuf, wbuf, Xf, r2, r3, Yp, Ps, zbuf, csem, xsem, wsem, osem):
        x16 = r3.bitcast(bf16); wb16 = wbuf.bitcast(bf16); o16 = r2.bitcast(bf16)
        mk=pltpu.make_async_copy
        ccopy = mk(c_hbm, cbuf, csem.at[0])
        def wcopy(et,i):
            return mk(w_hbm.at[i,:,pl.ds(et*128,128)], wb16.at[et,pl.ds(pl.multiple_of(i*(2*SI),8),D),:], wsem.at[et])
        def startW(et):
            @pl.loop(0,K)
            def _(i): wcopy(et,i).start()
        def waitW(et):
            @pl.loop(0,K)
            def _(i): wcopy(et,i).wait()
        def xcopy(b,dt,p):
            n=TP if p<NP-1 else TL
            t0=p*TP
            row0=pl.multiple_of((b*2+dt)*(2*MP)+64+t0,8)
            return mk(x_hbm.at[b,pl.ds(t0,n),pl.ds(dt*128,128)], x16.at[pl.ds(row0,n),:], xsem.at[b*2+dt,p])
        def xstart(g):
            b,p=divmod(g,NP)
            for dt in range(2): xcopy(b,dt,p).start()
        NO=NJ//UI
        def ocp(b,c,o):
            t0=o*UI*2*L; n=min(T,(o+1)*UI*2*L)-t0
            return mk(o16.at[pl.ds(pl.multiple_of(b*NJ*L*2+t0,8),n),:], out_hbm.at[b,pl.ds(t0,n),pl.ds(pl.multiple_of(c*128,128),128)], osem.at[b,o])

        ccopy.start()
        startW(0)
        zero = jnp.zeros
        for s in range(B*2):
            r3[pl.ds(s*MP,32),:] = zero((32,128),i32)
            r3[pl.ds(s*MP+32+M,MP-32-M),:] = zero((MP-32-M,128),i32)
        for et in (0,2):
            wbuf[et,pl.ds(K*SI,(32-K)*SI),:] = zero(((32-K)*SI,128),i32)
        if not vpu:
            for et in (1,3):
                wbuf[et,pl.ds(K*SI,(32-K)*SI),:] = zero(((32-K)*SI,128),i32)
        zbuf[...]=zero((8,128),i32)
        ccopy.wait()
        GWr = lambda: bc(cbuf[0:256,:],bf16)
        FAr = lambda: bc(cbuf[256:320,:],bf16)
        IAr = lambda: bc(cbuf[320:368,:],bf16)

        def wgroup(et,e2,g):
            tiles=[]
            for qp in range(4):
                q0 = g*8+qp*2
                t = jnp.concatenate([wbuf[et,pl.ds(q0,32,stride=SI),:], wbuf[et,pl.ds(q0+1,32,stride=SI),:]],axis=0)
                tiles.append(bc(t,bf16))
            o = jnp.dot(GWr(), jnp.concatenate(tiles,axis=1), preferred_element_type=f32)
            for qp in range(4):
                col = qp*128
                for qs in range(2):
                    q = g*8+qp*2+qs
                    for kg in range(8):
                        base=qs*256+kg*32
                        r0=o[base:base+8,col:col+128]; r1=o[base+8:base+16,col:col+128]
                        i0=o[base+16:base+24,col:col+128]; i1=o[base+24:base+32,col:col+128]
                        r2[pl.ds(e2*128*SW+q*SW+kg*8,8),:] = pack(r0,r1)
                        r2[pl.ds(e2*128*SW+q*SW+64+kg*8,8),:] = pack(i0-r0,i1-r1)
                        r2[pl.ds(e2*128*SW+q*SW+128+kg*8,8),:] = pack(r0+i0,r1+i1)
        def phaseW0():
            for e2 in range(2):
                et=2*e2
                waitW(et)
                if e2==0:
                    startW(2); xstart(0)
                else:
                    xstart(2)
                @pl.loop(0,2)
                def _(h):
                    if e2==0:
                        @pl.when(h==1)
                        def _(): xstart(1)
                    else:
                        @pl.when(h==1)
                        def _(): xstart(3)
                    for u in range(8): wgroup(et,e2,h*8+u)

        def fblock(b,j):
            tiles=[]
            for dt in range(2):
                X = r3[pl.ds((b*2+dt)*MP+j*L,N),:]
                top=X[0:64]; bot=X[64:128]
                E = (top & 0xFFFF) | (bot<<16)
                O = lax.shift_right_logical(top,16) | (bot & jnp.int32(-65536))
                tiles += [bc(E,bf16), bc(O,bf16)]
            Y = jnp.dot(FAr(), jnp.concatenate(tiles,axis=1), preferred_element_type=f32)
            J = b*NJ+j
            for dt in range(2):
                Ye=Y[:,dt*256:dt*256+128]; Yo=Y[:,dt*256+128:dt*256+256]
                Xf[dt,pl.ds(J*SX,64),:] = pack(Ye[:64]+Ye[64:], Yo[:64]+Yo[64:])
                Xf[dt,pl.ds(J*SX+64,64),:] = pack(Ye[:64],Yo[:64])
                Xf[dt,pl.ds(J*SX+128,64),:] = pack(Ye[64:],Yo[64:])
        nw=4
        def phaseF():
            @pl.loop(0,B)
            def _(b):
                for p in range(NP):
                    @pl.when(b==0)
                    def _(): xstart(p+nw)
                    if p==0:
                        @pl.when(b==1)
                        def _(): startW(1)
                    if p==1:
                        @pl.when(b==1)
                        def _(): startW(3)
                    for dt in range(2): xcopy(b,dt,p).wait()
                    for u in range(JP): fblock(b,p*JP+u)

        def wvpu_pieces(et,e2,qv,slot):
            pb=slot*2048
            pieces=[]
            def p1(r,poss):
                def run(tok):
                    taps=[r+8*a for a in range(4)]
                    words=[wbuf[et,pl.ds(i*SI+qv*8,8),:] if i<K else None for i in taps]
                    if tok is not None: words=[None if wd is None else wd|tok for wd in words]
                    for pos in poss:
                        u=[None if wd is None else pltpu.unpack_elementwise(wd,index=pos,packed_dtype=bf16,unpacked_dtype=f32) for wd in words]
                        Pv=pass1(u)
                        for kp in range(8):
                            z=Pv[kp] if r==0 else cmul(Pv[kp],-2*np.pi*(kp+0.5)/N*r)
                            base=pb+((kp*2+pos)*8+r)*16
                            Ps[pl.ds(base,8),:]=z[0]
                            Ps[pl.ds(base+8,8),:]=z[1]
                return run
            def p2(kp,odd):
                def run(tok):
                    outs=[]
                    for pos in range(2):
                        base=pb+((kp*2+pos)*8)*16
                        Q=[[Ps[pl.ds(base+r*16,8),:],Ps[pl.ds(base+r*16+8,8),:]] for r in range(8)]
                        if tok is not None:
                            for r in TOKR:
                                for h in TOKH: Q[r][h]=bc(bc(Q[r][h],i32)|tok,f32)
                        res=p2half(Q,odd)
                        o={}
                        for s_,(Re,Im,Re2,Ai,Bi,nBi) in res.items():
                            o[kp+16*s_]=(Re,Im-Re,Re+Im)
                            km=127-kp-16*(s_+4)
                            if nBi is None:
                                nIm2=Bi-Ai
                                o[km]=(Re2,nIm2-Re2,Re2+nIm2)
                            else:
                                pIm2=nBi+Ai
                                o[km]=(Re2,(0.0-pIm2)-Re2 if False else -(pIm2+Re2),Re2-pIm2)
                        outs.append(o)
                    for k in outs[0]:
                        for v in range(3):
                            r3[pl.ds(e2*(192*128)+(v*64+k)*128+qv*8,8),:]=pack(outs[0][k][v],outs[1][k][v])
                return run
            for r in range(8):
                if P1SPLIT:
                    for pos in range(2): pieces.append(p1(r,(pos,)))
                else: pieces.append(p1(r,(0,1)))
            for kp in range(8):
                for odd in range(2): pieces.append(p2(kp,odd))
            return pieces

        def mbin(k,c):
            def lhs(v): return jnp.concatenate([bc(Xf[dt,pl.ds(v*64+k,NR,stride=SX),:],bf16) for dt in range(2)],axis=1)
            if c==0:
                def rhs(v): return jnp.concatenate([bc(r2[pl.ds(e2*128*SW+v*64+k,128,stride=SW),:],bf16) for e2 in range(2)],axis=1)
            else:
                def rhs(v): return jnp.concatenate([bc(r3[pl.ds(pl.multiple_of(e2*(192*128)+(v*64+k)*128,8),128),:],bf16) for e2 in range(2)],axis=1)
            k1=jnp.dot(lhs(0),rhs(0),preferred_element_type=f32)
            k2=jnp.dot(lhs(1),rhs(1),preferred_element_type=f32)
            k3=jnp.dot(lhs(2),rhs(2),preferred_element_type=f32)
            Yr=k1-k3; Yi=k1+k2
            for e2 in range(2):
                Yp[e2,pl.ds(k*SY,2*NR),:] = pack(Yr[:,e2*128:e2*128+128],Yi[:,e2*128:e2*128+128])
            return [k1,k2,k3]
        def phaseM0():
            WP=UM//2
            waitW(1); waitW(3)
            @pl.loop(0,NK//UM)
            def _(kk):
                zm=zbuf[...]
                for u in range(WP):
                    wp=kk*WP+u
                    e2=wp//16; qv=wp%16
                    ks=mbin(kk*UM+2*u,0)+mbin(kk*UM+2*u+1,0)
                    if vpu:
                        ps=wvpu_pieces(1+2*e2,e2,qv,u%2)
                        n=len(ps)
                        for j,p in enumerate(ps):
                            pos=int(round(LAG+(j*(6*42-LAG-TAIL))/(n-1)))
                            pos=min(pos,6*42-1)
                            d,g=divmod(pos,42)
                            d=DORD[d]
                            tok=(bc(ks[d][g*8:g*8+8,0:128],i32)&zm) if TOK else None
                            p(tok)
        def phaseM1(UM1):
            @pl.loop(0,NK//UM1)
            def _(kk):
                for u in range(UM1): mbin(kk*UM1+u,1)

        def iblock(b,j):
            J=b*NJ+j
            tiles=[]
            for p in range(2):
                for e2 in range(2):
                    tiles.append(bc(Yp[e2,pl.ds(2*J+p,64,stride=SY),:],bf16))
            h = jnp.dot(IAr(), jnp.concatenate(tiles,axis=1), preferred_element_type=f32)
            oe = jnp.tanh(h[:,0:128])*(jnp.tanh(h[:,128:256]*0.5)*0.5+0.5)
            oo = jnp.tanh(h[:,256:384])*(jnp.tanh(h[:,384:512]*0.5)*0.5+0.5)
            r2[pl.ds(b*NJ*L+j*L,L),:] = pack(oe,oo)
        def phaseI(c):
            @pl.loop(0,B)
            def _(b):
                for o in range(NO):
                    for u in range(UI): iblock(b,o*UI+u)
                    ocp(b,c,o).start()

        with scope('W'): phaseW0()
        with scope('F'): phaseF()
        with scope('M0'): phaseM0()
        with scope('I0'): phaseI(0)
        with scope('M1'): phaseM1(16)
        for b in range(B):
            for o in range(NO): ocp(b,0,o).wait()
        with scope('I1'): phaseI(1)
        with scope('end'):
            for b in range(B):
                for o in range(NO): ocp(b,1,o).wait()

    cst = consts(K)
    def f(x,w):
        return pl.pallas_call(kernel,
            out_shape=jax.ShapeDtypeStruct((B,T,D),bf16),
            in_specs=[pl.BlockSpec(memory_space=pl.ANY)]*3,
            out_specs=pl.BlockSpec(memory_space=pl.ANY),
            scratch_shapes=[pltpu.VMEM(cst.shape,i32), pltpu.VMEM((4,32*SI,128),i32),
                            pltpu.VMEM((2,NR*SX,128),i32), pltpu.VMEM((R2,128),i32), pltpu.VMEM((R3,128),i32),
                            pltpu.VMEM((2,NK*SY,128),i32), pltpu.VMEM((2*2048+2*1536,128),f32), pltpu.VMEM((8,128),i32),
                            pltpu.SemaphoreType.DMA((1,)),
                            pltpu.SemaphoreType.DMA((B*2,NP)), pltpu.SemaphoreType.DMA((4,)), pltpu.SemaphoreType.DMA((B,NJ//UI))],
            compiler_params=pltpu.CompilerParams(vmem_limit_bytes=127*1024*1024, flags=flags),
        )(x,w,jnp.asarray(cst))
    return f


@jax.jit
def pallas_standalone__autoregressive_conv_wavernn__speech_kernel(x: jax.Array, w: jax.Array):
    B, T, D = x.shape
    K = w.shape[0]
    return make(B, T, D, K, scopes=False, UM=8, TOKR=(0, 1, 2, 3))(x, w)
```

```python
import contextlib
import numpy as np
import jax, jax.numpy as jnp
from jax import lax
from jax.experimental import pallas as pl
from jax.experimental.pallas import tpu as pltpu
import ml_dtypes

N = 128
L = 96
NK = 64
NU = 63
SX = 196; SW = 196; SI = 132; SY = 340


def _pack_rows(a):
    u = a.astype(np.float32).astype(ml_dtypes.bfloat16).view(np.uint16).astype(np.uint32)
    return (u[0::2] | (u[1::2] << 16)).view(np.int32)


def consts(K):
    m = L + K - 1
    assert m == 2 * (NU - 1) + 2
    th = 2 * np.pi * (np.arange(NK) + 0.5) / N
    ks = np.arange(1, NU)
    z = np.concatenate([np.exp(-1j * th[ks]), np.exp(1j * th[ks]), [1.0, -1.0]])
    V = z[:, None] ** np.arange(m)[None]
    BT = np.linalg.inv(V).T
    off = 32 - (K - 1)
    F = np.zeros((128, N))
    F[ks, off:off + m] = BT[:NU - 1].real
    F[64 + ks, off:off + m] = BT[:NU - 1].imag
    bp, bm = BT[-2].real, BT[-1].real
    F[0, off:off + m] = (bp + bm) / 2
    F[64, off:off + m] = (bp - bm) / 2
    Fp = np.zeros_like(F); Fp[:, 0::2] = F[:, :64]; Fp[:, 1::2] = F[:, 64:]
    i = np.arange(32)
    Gc = np.cos(th[:, None] * i[None]); Gs = -np.sin(th[:, None] * i[None])
    Gc[0] = (i % 2 == 0); Gs[0] = (i % 2 == 1)
    Gc[NU:] = 0; Gs[NU:] = 0
    Gc[:, K:] = 0; Gs[:, K:] = 0
    GW = np.zeros((512, 128))
    for qs in range(2):
        for kg in range(8):
            base = qs * 256 + kg * 32
            for h, (G, dpar) in enumerate([(Gc, 0), (Gc, 1), (Gs, 0), (Gs, 1)]):
                GW[base + h * 8:base + h * 8 + 8, 2 * (qs * 32 + i) + dpar] = G[kg * 8:kg * 8 + 8, :]
    r = np.arange(L)
    IA = np.zeros((L, 128))
    IA[:, 0::2] = 2 * np.cos(r[:, None] * th[None]); IA[:, 1::2] = 2 * np.sin(r[:, None] * th[None])
    IA[:, 0] = 1 + (-1.0) ** r; IA[:, 1] = 1 - (-1.0) ** r
    IA[:, 2 * NU:] = 0
    sgn = np.ones((8, 128), np.float32); sgn[0] = -1
    return np.concatenate([_pack_rows(GW), _pack_rows(Fp), _pack_rows(IA), sgn.view(np.int32)], 0)


def f32c(v): return float(np.float32(v))
def pass1(u):
    out = [None] * 8
    for kp in range(4):
        ph = 2 * np.pi * (kp + 0.5) / 16
        c1, s1 = np.cos(ph), -np.sin(ph); c2, s2 = np.cos(2 * ph), -np.sin(2 * ph); c3, s3 = np.cos(3 * ph), -np.sin(3 * ph)
        Er = u[0] + u[2] * f32c(c2); Ei = u[2] * f32c(s2)
        if u[3] is not None:
            Or = u[1] * f32c(c1) + u[3] * f32c(c3); Oi = u[1] * f32c(s1) + u[3] * f32c(s3)
        else:
            Or = u[1] * f32c(c1); Oi = u[1] * f32c(s1)
        out[kp] = (Er + Or, Ei + Oi)
        out[7 - kp] = (Er - Or, Oi - Ei)
    return out
def cmul(z, ang):
    c, s = f32c(np.cos(ang)), f32c(np.sin(ang))
    return (z[0] * c - z[1] * s, z[0] * s + z[1] * c)
def p2half(Q, odd, kp):
    def half(x):
        if not odd:
            a = (x[0][0] + x[2][0], x[0][1] + x[2][1]); c = (x[1][0] + x[3][0], x[1][1] + x[3][1])
            return {0: (a[0] + c[0], a[1] + c[1]), 2: (a[0] - c[0], a[1] - c[1])}
        b = (x[0][0] - x[2][0], x[0][1] - x[2][1]); d = (x[1][0] - x[3][0], x[1][1] - x[3][1])
        return {1: (b[0] + d[1], b[1] - d[0]), 3: (b[0] - d[1], b[1] + d[0])}
    A = half([Q[0], Q[2], Q[4], Q[6]]); Bv = half([Q[1], Q[3], Q[5], Q[7]])
    h = f32c(np.sqrt(0.5)); o = {}
    for s in A:
        Ar, Ai = A[s]; br, bi = Bv[s]
        k = kp + 16 * s; km = 127 - kp - 16 * (s + 4)
        if s == 0:   Br, Bi, nBi = br, bi, None
        elif s == 1: Br, Bi, nBi = (br + bi) * h, (bi - br) * h, None
        elif s == 2: Br, Bi, nBi = bi, None, br
        else:        Br, Bi, nBi = (bi - br) * h, None, (br + bi) * h
        if 0 < k < NU:
            Re = Ar + Br
            Im = Ai + Bi if nBi is None else Ai - nBi
            o[k] = (Re, Im - Re, Re + Im)
        if 0 < km < NU:
            Re2 = Ar - Br
            if nBi is None:
                nIm2 = Bi - Ai
                o[km] = (Re2, nIm2 - Re2, Re2 + nIm2)
            else:
                pIm2 = nBi + Ai
                o[km] = (Re2, -(pIm2 + Re2), Re2 - pIm2)
    return o


def make(B, T, D, K, UI=14, NI0=7, UM1=21, scopes=True, flags=None, TOKR=(0, 1, 2, 3), NP=4, NX0=1, LAG=0, TAIL=8):
    M = T // 2; NJ = -(-M // L); MP = (NJ - 1) * L + N; NR = B * NJ
    f32 = jnp.float32; bf16 = jnp.bfloat16; i32 = jnp.int32
    JP = NJ // NP; TP = JP * 2 * L; TL = T - (NP - 1) * TP
    UM0 = NU // NI0; WP0 = -(-32 // NI0)
    assert NJ % NP == 0 and NJ % UI == 0 and NU % NI0 == 0 and NU % UM1 == 0
    def bc(x, t): return pltpu.bitcast(x, t)
    def pack(a, b): return pltpu.pack_elementwise([a, b], packed_dtype=bf16)
    scope = jax.named_scope if scopes else (lambda n: contextlib.nullcontext())
    R3 = 2 * 192 * 128
    R2 = 2 * 128 * SW
    assert 4 * MP <= R3 and B * NJ * L <= R2
    H2 = D // 2
    PS = 2048 + 128
    NO = NJ // UI

    def kernel(x_hbm, w_hbm, c_hbm, out_hbm,
               cbuf, wbuf, wbuf1, Xf, r2, r3, Yp, Ps, zbuf, csem, xsem, wsem, osem, w1sem):
        x16 = r3.bitcast(bf16); wb16 = wbuf.bitcast(bf16); w116 = wbuf1.bitcast(bf16); o16 = r2.bitcast(bf16)
        mk = pltpu.make_async_copy
        mo = pl.multiple_of
        ccopy = mk(c_hbm, cbuf, csem.at[0])
        def wcopy(i, h):
            return mk(w_hbm.at[i, pl.ds(mo(h * H2, 8), H2), pl.ds(0, 128)],
                      wb16.at[0, pl.ds(mo(i * (2 * SI) + h * H2, 8), H2), :], wsem.at[h])
        def wcopyg(i):
            return mk(w_hbm.at[i, :, pl.ds(D, 128)], wb16.at[1, pl.ds(mo(i * (2 * SI), 8), D), :], wsem.at[2])
        def w1copy(qh):
            e2 = qh // 2; h = qh % 2
            return mk(w_hbm.at[:, pl.ds(mo(h * H2, 8), H2), pl.ds(mo((1 + 2 * e2) * 128, 128), 128)], w116.at[qh], w1sem.at[qh])
        def xcopy(b, dt, p):
            n = TP if p < NP - 1 else TL
            row0 = mo((b * 2 + dt) * (2 * MP) + 64 + p * TP, 8)
            return mk(x_hbm.at[b, pl.ds(p * TP, n), pl.ds(dt * 128, 128)], x16.at[pl.ds(row0, n), :], xsem.at[b * 2 + dt, p])
        def xstart(g):
            b, p = divmod(g, NP)
            for dt in range(2): xcopy(b, dt, p).start()
        def ocp(b, c, o):
            t0 = o * UI * 2 * L; n = min(T, (o + 1) * UI * 2 * L) - t0
            return mk(o16.at[pl.ds(mo(b * NJ * L * 2 + t0, 8), n), :],
                      out_hbm.at[b, pl.ds(t0, n), pl.ds(mo(c * 128, 128), 128)], osem.at[b, o])

        @pl.loop(0, K)
        def _(i): wcopy(i, 0).start()
        ccopy.start()
        @pl.loop(0, K)
        def _(i): wcopy(i, 1).start()
        @pl.loop(0, K)
        def _(i): wcopyg(i).start()
        for g in range(NX0): xstart(g)
        zero = jnp.zeros
        for s in range(B * 2):
            r3[pl.ds(s * MP, 32), :] = zero((32, 128), i32)
            r3[pl.ds(s * MP + 32 + M, MP - 32 - M), :] = zero((MP - 32 - M, 128), i32)
        for e2 in range(2):
            wbuf[e2, pl.ds(K * SI, (32 - K) * SI), :] = zero(((32 - K) * SI, 128), i32)
            Yp[e2, pl.ds(NU * SY, 2 * NR), :] = zero((2 * NR, 128), i32)
        zbuf[...] = zero((8, 128), i32)
        ccopy.wait()
        GWr = lambda: bc(cbuf[0:256, :], bf16)
        FAr = lambda: bc(cbuf[256:320, :], bf16)
        IAr = lambda: bc(cbuf[320:368, :], bf16)
        SGN = lambda: bc(cbuf[368:376, :], f32)

        def wgroup(e2, g):
            tiles = []
            for qp in range(4):
                q0 = g * 8 + qp * 2
                t = jnp.concatenate([wbuf[e2, pl.ds(q0, 32, stride=SI), :], wbuf[e2, pl.ds(q0 + 1, 32, stride=SI), :]], axis=0)
                tiles.append(bc(t, bf16))
            o = jnp.dot(GWr(), jnp.concatenate(tiles, axis=1), preferred_element_type=f32)
            sg = SGN()
            for qp in range(4):
                col = qp * 128
                for qs in range(2):
                    q = g * 8 + qp * 2 + qs
                    for kg in range(8):
                        base = qs * 256 + kg * 32
                        r0 = o[base:base + 8, col:col + 128]; r1 = o[base + 8:base + 16, col:col + 128]
                        i0 = o[base + 16:base + 24, col:col + 128]; i1 = o[base + 24:base + 32, col:col + 128]
                        j0, j1 = (i0 * sg, i1 * sg) if kg == 0 else (i0, i1)
                        row = e2 * 128 * SW + q * SW + kg * 8
                        r2[pl.ds(row, 8), :] = pack(r0, r1)
                        r2[pl.ds(row + 64, 8), :] = pack(i0 - r0, i1 - r1)
                        r2[pl.ds(row + 128, 8), :] = pack(r0 + j0, r1 + j1)
        def phaseW0():
            for e2 in range(2):
                for h in range(2):
                    if e2 == 0:
                        if h == 1:
                            for g in range(NX0, B * NP): xstart(g)
                            for qh in range(4): w1copy(qh).start()
                        for i in range(K): wcopy(i, h).wait()
                    elif h == 0:
                        for i in range(K): wcopyg(i).wait()
                    for u in range(8): wgroup(e2, h * 8 + u)

        def fblock(b, j):
            tiles = []
            for dt in range(2):
                X = r3[pl.ds((b * 2 + dt) * MP + j * L, N), :]
                top = X[0:64]; bot = X[64:128]
                E = (top & 0xFFFF) | (bot << 16)
                O = lax.shift_right_logical(top, 16) | (bot & jnp.int32(-65536))
                tiles += [bc(E, bf16), bc(O, bf16)]
            Y = jnp.dot(FAr(), jnp.concatenate(tiles, axis=1), preferred_element_type=f32)
            J = b * NJ + j
            for dt in range(2):
                Ye = Y[:, dt * 256:dt * 256 + 128]; Yo = Y[:, dt * 256 + 128:dt * 256 + 256]
                Xf[dt, pl.ds(J * SX, 64), :] = pack(Ye[:64] + Ye[64:], Yo[:64] + Yo[64:])
                Xf[dt, pl.ds(J * SX + 64, 64), :] = pack(Ye[:64], Yo[:64])
                Xf[dt, pl.ds(J * SX + 128, 64), :] = pack(Ye[64:], Yo[64:])
        def phaseF():
            @pl.loop(0, B)
            def _(b):
                for p in range(NP):
                    for dt in range(2): xcopy(b, dt, p).wait()
                    for u in range(JP): fblock(b, p * JP + u)

        def wvpu_pieces(wp, slot):
            e2 = wp // 16; qv = wp % 16
            pb = slot * PS
            out_row = lambda v, k: e2 * (192 * 128) + (v * 64 + k) * 128 + qv * 8
            pieces = []
            def p1(r, pos):
                def run(tok):
                    taps = [r + 8 * a for a in range(4)]
                    words = [wbuf1[e2 * 2 + qv // 8, i, pl.ds(mo((qv % 8) * 8, 8), 8), :] | tok if i < K else None for i in taps]
                    u = [None if wd is None else pltpu.unpack_elementwise(wd, index=pos, packed_dtype=bf16, unpacked_dtype=f32) for wd in words]
                    Pv = pass1(u)
                    for kp in range(8):
                        z = Pv[kp] if r == 0 else cmul(Pv[kp], -2 * np.pi * (kp + 0.5) / N * r)
                        base = pb + ((kp * 2 + pos) * 8 + r) * 16
                        Ps[pl.ds(base, 8), :] = z[0]
                        Ps[pl.ds(base + 8, 8), :] = z[1]
                    s = (u[0] + u[2]) + (u[1] + u[3] if u[3] is not None else u[1])
                    Ps[pl.ds(pb + 2048 + (pos * 8 + r) * 8, 8), :] = s
                return run
            def p2(kp, odd):
                def run(tok):
                    outs = []
                    for pos in range(2):
                        base = pb + ((kp * 2 + pos) * 8) * 16
                        Q = [[Ps[pl.ds(base + r * 16, 8), :], Ps[pl.ds(base + r * 16 + 8, 8), :]] for r in range(8)]
                        for r in TOKR:
                            for h in range(2): Q[r][h] = bc(bc(Q[r][h], i32) | tok, f32)
                        outs.append(p2half(Q, odd, kp))
                    for k in outs[0]:
                        for v in range(3):
                            r3[pl.ds(out_row(v, k), 8), :] = pack(outs[0][k][v], outs[1][k][v])
                return run
            def p3(tok):
                res = []
                for pos in range(2):
                    s = [Ps[pl.ds(pb + 2048 + (pos * 8 + r) * 8, 8), :] for r in range(8)]
                    s[0] = bc(bc(s[0], i32) | tok, f32); s[1] = bc(bc(s[1], i32) | tok, f32)
                    we = (s[0] + s[2]) + (s[4] + s[6]); wo = (s[1] + s[3]) + (s[5] + s[7])
                    res.append((we, wo - we, we - wo))
                for v in range(3):
                    r3[pl.ds(out_row(v, 0), 8), :] = pack(res[0][v], res[1][v])
            for r in range(8):
                for pos in range(2): pieces.append(p1(r, pos))
            pieces.append(p3)
            for kp in range(8):
                for odd in range(2): pieces.append(p2(kp, odd))
            return pieces

        def mbin(k, c):
            def lhs(v): return jnp.concatenate([bc(Xf[dt, pl.ds(v * 64 + k, NR, stride=SX), :], bf16) for dt in range(2)], axis=1)
            if c == 0:
                def rhs(v): return jnp.concatenate([bc(r2[pl.ds(e2 * 128 * SW + v * 64 + k, 128, stride=SW), :], bf16) for e2 in range(2)], axis=1)
            else:
                def rhs(v): return jnp.concatenate([bc(r3[pl.ds(mo(e2 * (192 * 128) + (v * 64 + k) * 128, 8), 128), :], bf16) for e2 in range(2)], axis=1)
            k1 = jnp.dot(lhs(0), rhs(0), preferred_element_type=f32)
            k2 = jnp.dot(lhs(1), rhs(1), preferred_element_type=f32)
            k3 = jnp.dot(lhs(2), rhs(2), preferred_element_type=f32)
            Yr = k1 - k3; Yi = k1 + k2
            for e2 in range(2):
                Yp[e2, pl.ds(k * SY, 2 * NR), :] = pack(Yr[:, e2 * 128:e2 * 128 + 128], Yi[:, e2 * 128:e2 * 128 + 128])
            return [k1, k2, k3]
        def phaseM0():
            RG = 2 * NR // 8; G = 3 * RG
            need = [(8 * q) // WP0 for q in range(4)]
            @pl.loop(0, NI0)
            def _(kk):
                for q in range(4):
                    @pl.when(kk == need[q])
                    def _(): w1copy(q).wait()
                zm = zbuf[...]
                ks = []
                for u in range(UM0): ks += mbin(kk * UM0 + u, 0)
                ps = []
                for u in range(WP0):
                    ps += wvpu_pieces(jnp.minimum(kk * WP0 + u, 31), u % 2)
                n = len(ps); lo = LAG; hi = UM0 * G - TAIL
                for j, p in enumerate(ps):
                    pos = min(int(round(lo + (j * (hi - lo)) / (n - 1))), UM0 * G - 1)
                    d, g = divmod(pos, RG)
                    p(bc(ks[d][g * 8:g * 8 + 8, 0:128], i32) & zm)
        def phaseM1():
            @pl.loop(0, NU // UM1)
            def _(kk):
                for u in range(UM1): mbin(kk * UM1 + u, 1)

        def iblock(b, j):
            J = b * NJ + j
            tiles = []
            for p in range(2):
                for e2 in range(2):
                    tiles.append(bc(Yp[e2, pl.ds(2 * J + p, 64, stride=SY), :], bf16))
            h = jnp.dot(IAr(), jnp.concatenate(tiles, axis=1), preferred_element_type=f32)
            oe = jnp.tanh(h[:, 0:128]) * (jnp.tanh(h[:, 128:256] * 0.5) * 0.5 + 0.5)
            oo = jnp.tanh(h[:, 256:384]) * (jnp.tanh(h[:, 384:512] * 0.5) * 0.5 + 0.5)
            r2[pl.ds(b * NJ * L + j * L, L), :] = pack(oe, oo)
        def phaseI(c):
            @pl.loop(0, B)
            def _(b):
                for o in range(NO):
                    for u in range(UI): iblock(b, o * UI + u)
                    ocp(b, c, o).start()

        with scope('W'): phaseW0()
        with scope('F'): phaseF()
        @pl.loop(0, 2)
        def _(c):
            @pl.when(c == 0)
            def _():
                with scope('M0'): phaseM0()
            @pl.when(c == 1)
            def _():
                with scope('M1'): phaseM1()
                for b in range(B):
                    for o in range(NO): ocp(b, 0, o).wait()
            with scope('I'): phaseI(c)
        with scope('end'):
            for b in range(B):
                for o in range(NO): ocp(b, 1, o).wait()

    cst = consts(K)
    def f(x, w):
        return pl.pallas_call(kernel,
            out_shape=jax.ShapeDtypeStruct((B, T, D), bf16),
            in_specs=[pl.BlockSpec(memory_space=pl.ANY)] * 3,
            out_specs=pl.BlockSpec(memory_space=pl.ANY),
            scratch_shapes=[pltpu.VMEM(cst.shape, i32), pltpu.VMEM((2, 32 * SI, 128), i32), pltpu.VMEM((4, K, 64, 128), i32),
                            pltpu.VMEM((2, NR * SX, 128), i32), pltpu.VMEM((R2, 128), i32), pltpu.VMEM((R3, 128), i32),
                            pltpu.VMEM((2, NK * SY, 128), i32), pltpu.VMEM((2 * PS, 128), f32), pltpu.VMEM((8, 128), i32),
                            pltpu.SemaphoreType.DMA((1,)), pltpu.SemaphoreType.DMA((B * 2, NP)), pltpu.SemaphoreType.DMA((3,)),
                            pltpu.SemaphoreType.DMA((B, NO)), pltpu.SemaphoreType.DMA((4,))],
            compiler_params=pltpu.CompilerParams(vmem_limit_bytes=127 * 1024 * 1024, flags=flags),
        )(x, w, jnp.asarray(cst))
    return f


@jax.jit
def pallas_standalone__autoregressive_conv_wavernn__speech_kernel(x: jax.Array, w: jax.Array):
    B, T, D = x.shape
    K = w.shape[0]
    return make(B, T, D, K, scopes=False)(x, w)
```

```python
import contextlib
import numpy as np
import jax, jax.numpy as jnp
from jax import lax
from jax.experimental import pallas as pl
from jax.experimental.pallas import tpu as pltpu
import ml_dtypes

N = 128
L = 96
NK = 64
NU = 63
SX = 196; SW = 196; SI = 132; SY = 340


def _pack_rows(a):
    u = a.astype(np.float32).astype(ml_dtypes.bfloat16).view(np.uint16).astype(np.uint32)
    return (u[0::2] | (u[1::2] << 16)).view(np.int32)


def consts(K):
    m = L + K - 1
    assert m == 2 * (NU - 1) + 2
    th = 2 * np.pi * (np.arange(NK) + 0.5) / N
    ks = np.arange(1, NU)
    z = np.concatenate([np.exp(-1j * th[ks]), np.exp(1j * th[ks]), [1.0, -1.0]])
    V = z[:, None] ** np.arange(m)[None]
    BT = np.linalg.inv(V).T
    off = 32 - (K - 1)
    F = np.zeros((128, N))
    F[ks, off:off + m] = 2 * BT[:NU - 1].real
    F[64 + ks, off:off + m] = 2 * BT[:NU - 1].imag
    bp, bm = BT[-2].real, BT[-1].real
    F[0, off:off + m] = bp + bm
    F[64, off:off + m] = bp - bm
    Fp = np.zeros_like(F); Fp[:, 0::2] = F[:, :64]; Fp[:, 1::2] = F[:, 64:]
    i = np.arange(32)
    Gc = np.cos(th[:, None] * i[None]); Gs = -np.sin(th[:, None] * i[None])
    Gc[0] = (i % 2 == 0); Gs[0] = (i % 2 == 1)
    Gc[NU:] = 0; Gs[NU:] = 0
    Gc[:, K:] = 0; Gs[:, K:] = 0
    GW = np.zeros((512, 128))
    for qs in range(2):
        for kg in range(8):
            base = qs * 256 + kg * 32
            for h, (G, dpar) in enumerate([(Gc, 0), (Gc, 1), (Gs, 0), (Gs, 1)]):
                GW[base + h * 8:base + h * 8 + 8, 2 * (qs * 32 + i) + dpar] = G[kg * 8:kg * 8 + 8, :]
    r = np.arange(L)
    IA = np.zeros((L, 128))
    IA[:, 0::2] = np.cos(r[:, None] * th[None]); IA[:, 1::2] = np.sin(r[:, None] * th[None])
    IA[:, 0] = (1 + (-1.0) ** r) / 2; IA[:, 1] = (1 - (-1.0) ** r) / 2
    IA[:, 2 * NU:] = 0
    sgn = np.ones((8, 128), np.float32); sgn[0] = -1
    return np.concatenate([_pack_rows(GW), _pack_rows(Fp), _pack_rows(IA), sgn.view(np.int32)], 0)


def f32c(v): return float(np.float32(v))
def pass1(u):
    out = [None] * 8
    for kp in range(4):
        ph = 2 * np.pi * (kp + 0.5) / 16
        c1, s1 = np.cos(ph), -np.sin(ph); c2, s2 = np.cos(2 * ph), -np.sin(2 * ph); c3, s3 = np.cos(3 * ph), -np.sin(3 * ph)
        Er = u[0] + u[2] * f32c(c2); Ei = u[2] * f32c(s2)
        if u[3] is not None:
            Or = u[1] * f32c(c1) + u[3] * f32c(c3); Oi = u[1] * f32c(s1) + u[3] * f32c(s3)
        else:
            Or = u[1] * f32c(c1); Oi = u[1] * f32c(s1)
        out[kp] = (Er + Or, Ei + Oi)
        out[7 - kp] = (Er - Or, Oi - Ei)
    return out
def cmul(z, ang):
    c, s = f32c(np.cos(ang)), f32c(np.sin(ang))
    return (z[0] * c - z[1] * s, z[0] * s + z[1] * c)
def p2half(Q, odd, kp):
    def half(x):
        if not odd:
            a = (x[0][0] + x[2][0], x[0][1] + x[2][1]); c = (x[1][0] + x[3][0], x[1][1] + x[3][1])
            return {0: (a[0] + c[0], a[1] + c[1]), 2: (a[0] - c[0], a[1] - c[1])}
        b = (x[0][0] - x[2][0], x[0][1] - x[2][1]); d = (x[1][0] - x[3][0], x[1][1] - x[3][1])
        return {1: (b[0] + d[1], b[1] - d[0]), 3: (b[0] - d[1], b[1] + d[0])}
    A = half([Q[0], Q[2], Q[4], Q[6]]); Bv = half([Q[1], Q[3], Q[5], Q[7]])
    h = f32c(np.sqrt(0.5)); o = {}
    for s in A:
        Ar, Ai = A[s]; br, bi = Bv[s]
        k = kp + 16 * s; km = 127 - kp - 16 * (s + 4)
        if s == 0:   Br, Bi, nBi = br, bi, None
        elif s == 1: Br, Bi, nBi = (br + bi) * h, (bi - br) * h, None
        elif s == 2: Br, Bi, nBi = bi, None, br
        else:        Br, Bi, nBi = (bi - br) * h, None, (br + bi) * h
        if 0 < k < NU:
            Re = Ar + Br
            Im = Ai + Bi if nBi is None else Ai - nBi
            o[k] = (Re, Im - Re, Re + Im)
        if 0 < km < NU:
            Re2 = Ar - Br
            if nBi is None:
                nIm2 = Bi - Ai
                o[km] = (Re2, nIm2 - Re2, Re2 + nIm2)
            else:
                pIm2 = nBi + Ai
                o[km] = (Re2, -(pIm2 + Re2), Re2 - pIm2)
    return o

def _add(a, b): return b if a is None else (a if b is None else a + b)
def _sub(a, b): return a if b is None else (-b if a is None else a - b)
def cadd(x, y):
    if x is None: return y
    if y is None: return x
    return (x[0] + y[0], x[1] + y[1])
def csub(x, y):
    if y is None: return x
    if x is None: return (-y[0], -y[1])
    return (x[0] - y[0], x[1] - y[1])
def dft4c(x0, x1, y2, y3):
    c = (x1[0] + y3[0], x1[1] - y3[1]); d = (x1[0] - y3[0], x1[1] + y3[1])
    if x0 is None:
        assert y2 is None
        return [c, (d[1], -d[0]), (-c[0], -c[1]), (-d[1], d[0])]
    a = (x0[0] + y2[0], x0[1] - y2[1]); b = (x0[0] - y2[0], x0[1] + y2[1])
    return [(a[0] + c[0], a[1] + c[1]), (b[0] + d[1], b[1] - d[0]), (a[0] - c[0], a[1] - c[1]), (b[0] - d[1], b[1] + d[0])]
def dft8(x):
    A = dft4c(x[0], x[2], x[4], x[6]); Bv = dft4c(x[1], x[3], x[5], x[7])
    h = f32c(np.sqrt(0.5))
    b0, b1, b2, b3 = Bv
    t1 = ((b1[0] + b1[1]) * h, (b1[1] - b1[0]) * h)
    out = [None] * 8
    out[0] = (A[0][0] + b0[0], A[0][1] + b0[1]); out[4] = (A[0][0] - b0[0], A[0][1] - b0[1])
    out[1] = (A[1][0] + t1[0], A[1][1] + t1[1]); out[5] = (A[1][0] - t1[0], A[1][1] - t1[1])
    out[2] = (A[2][0] + b2[1], A[2][1] - b2[0]); out[6] = (A[2][0] - b2[1], A[2][1] + b2[0])
    u3 = (b3[1] - b3[0]) * h; v3 = (b3[0] + b3[1]) * h
    out[3] = (A[3][0] + u3, A[3][1] - v3); out[7] = (A[3][0] - u3, A[3][1] + v3)
    return out
def inv6(P):
    h = f32c(np.sqrt(0.5)); y = [None] * 6
    for par in range(2):
        R = []
        for k in range(2):
            x, z = P[k], P[3 - k]
            if par == 0: v = (x[0] + z[0], x[1] - z[1])
            else:
                v = (x[0] - z[0], x[1] + z[1]); v = cmul(v, -2 * np.pi * (k + 0.5) / 8)
            R.append(v)
        (r0, i0), (r1, i1) = R
        y[par] = r0 + r1
        y[par + 2] = ((r0 + i0) + (i1 - r1)) * h
        y[par + 4] = i0 - i1
    return y
def invB(Q, odd):
    P = []
    for k in range(4):
        x, z = Q[k], Q[7 - k]
        if not odd: P.append((x[0] + z[0], x[1] - z[1]))
        else: P.append(cmul((x[0] - z[0], x[1] + z[1]), -2 * np.pi * (k + 0.5) / 16))
    return inv6(P)


def make(B, T, D, K, UI=14, NI0=7, NI1=7, SP=2, scopes=True, flags=None, TOKR=(0, 1, 2, 3), NP=4, NX0=1, LAG=0, TAIL=8, TAIL1=40, DBG=''):
    M = T // 2; NJ = -(-M // L); MP = (NJ - 1) * L + N; NR = B * NJ
    f32 = jnp.float32; bf16 = jnp.bfloat16; i32 = jnp.int32
    JP = NJ // NP; TP = JP * 2 * L; TL = T - (NP - 1) * TP
    UM0 = NU // NI0; WP0 = -(-32 // NI0)
    UM1 = NU // NI1; NSP = NI1 * SP; JM = NR - 8 * NSP
    assert 0 < JM <= NR and JM % 4 == 0
    JH = NR - JM
    def odd4(n): return n + 4 if n % 8 == 0 else n
    SA = odd4(2 * JM); SB = odd4(2 * JH)
    def pieces_of(J0, J1, sem0):
        out = []; J = J0
        while J < J1:
            n = min(UI, J1 - J, NJ - J % NJ); out.append((J, n, sem0 + len(out))); J += n
        return out
    PCA = pieces_of(0, JM, 0); PCC = pieces_of(JM, NR, len(PCA))
    assert NJ % NP == 0 and NJ % UI == 0 and NU % NI0 == 0 and NU % UM1 == 0
    def bc(x, t): return pltpu.bitcast(x, t)
    def pack(a, b): return pltpu.pack_elementwise([a, b], packed_dtype=bf16)
    scope = jax.named_scope if scopes else (lambda n: contextlib.nullcontext())
    R3 = 2 * 192 * 128
    R2 = 2 * 128 * SW
    assert 4 * MP <= R3 and B * NJ * L <= R2
    H2 = D // 2
    PS = 2048 + 128; PV = 4096
    OC = B * NJ * L
    assert OC + 2 * NK * SB <= R2
    NO = NJ // UI

    def kernel(x_hbm, w_hbm, c_hbm, out_hbm,
               cbuf, wbuf, wbuf1, Xf, r2, r3, Ya, Yb, vbuf, Ps, zbuf, csem, xsem, wsem, osem, w1sem, vsem):
        x16 = r3.bitcast(bf16); wb16 = wbuf.bitcast(bf16); w116 = wbuf1.bitcast(bf16); o16 = r2.bitcast(bf16); v16 = vbuf.bitcast(bf16)
        mk = pltpu.make_async_copy
        mo = pl.multiple_of
        ccopy = mk(c_hbm, cbuf, csem.at[0])
        def wcopy(i, h):
            return mk(w_hbm.at[i, pl.ds(mo(h * H2, 8), H2), pl.ds(0, 128)],
                      wb16.at[0, pl.ds(mo(i * (2 * SI) + h * H2, 8), H2), :], wsem.at[h])
        def wcopyg(i):
            return mk(w_hbm.at[i, :, pl.ds(D, 128)], wb16.at[1, pl.ds(mo(i * (2 * SI), 8), D), :], wsem.at[2])
        def w1copy(qh):
            e2 = qh // 2; h = qh % 2
            return mk(w_hbm.at[:, pl.ds(mo(h * H2, 8), H2), pl.ds(mo((1 + 2 * e2) * 128, 128), 128)], w116.at[qh], w1sem.at[qh])
        def xcopy(b, dt, p):
            n = TP if p < NP - 1 else TL
            row0 = mo((b * 2 + dt) * (2 * MP) + 64 + p * TP, 8)
            return mk(x_hbm.at[b, pl.ds(p * TP, n), pl.ds(dt * 128, 128)], x16.at[pl.ds(row0, n), :], xsem.at[b * 2 + dt, p])
        def xstart(g):
            b, p = divmod(g, NP)
            for dt in range(2): xcopy(b, dt, p).start()
        def ocp(pc, c):
            J, nb, si = pc; b, j = divmod(J, NJ)
            t0 = j * 2 * L; n = min(T, (j + nb) * 2 * L) - t0
            return mk(o16.at[pl.ds(J * 2 * L, n), :], out_hbm.at[b, pl.ds(t0, n), pl.ds(mo(c * 128, 128), 128)], osem.at[si])

        @pl.loop(0, K)
        def _(i): wcopy(i, 0).start()
        ccopy.start()
        @pl.loop(0, K)
        def _(i): wcopy(i, 1).start()
        @pl.loop(0, K)
        def _(i): wcopyg(i).start()
        for g in range(NX0): xstart(g)
        zero = jnp.zeros
        for s in range(B * 2):
            r3[pl.ds(s * MP, 32), :] = zero((32, 128), i32)
            r3[pl.ds(s * MP + 32 + M, MP - 32 - M), :] = zero((MP - 32 - M, 128), i32)
        for e2 in range(2):
            wbuf[e2, pl.ds(K * SI, (32 - K) * SI), :] = zero(((32 - K) * SI, 128), i32)
            Ya[e2, pl.ds(NU * SA, 2 * JM), :] = zero((2 * JM, 128), i32)
        zbuf[...] = zero((8, 128), i32)
        ccopy.wait()
        GWr = lambda: bc(cbuf[0:256, :], bf16)
        FAr = lambda: bc(cbuf[256:320, :], bf16)
        IAr = lambda: bc(cbuf[320:368, :], bf16)
        SGN = lambda: bc(cbuf[368:376, :], f32)

        def wgroup(e2, g):
            tiles = []
            for qp in range(4):
                q0 = g * 8 + qp * 2
                t = jnp.concatenate([wbuf[e2, pl.ds(q0, 32, stride=SI), :], wbuf[e2, pl.ds(q0 + 1, 32, stride=SI), :]], axis=0)
                tiles.append(bc(t, bf16))
            o = jnp.dot(GWr(), jnp.concatenate(tiles, axis=1), preferred_element_type=f32)
            sg = SGN()
            for qp in range(4):
                col = qp * 128
                for qs in range(2):
                    q = g * 8 + qp * 2 + qs
                    for kg in range(8):
                        base = qs * 256 + kg * 32
                        r0 = o[base:base + 8, col:col + 128]; r1 = o[base + 8:base + 16, col:col + 128]
                        i0 = o[base + 16:base + 24, col:col + 128]; i1 = o[base + 24:base + 32, col:col + 128]
                        j0, j1 = (i0 * sg, i1 * sg) if kg == 0 else (i0, i1)
                        row = e2 * 128 * SW + q * SW + kg * 8
                        r2[pl.ds(row, 8), :] = pack(r0, r1)
                        r2[pl.ds(row + 64, 8), :] = pack(i0 - r0, i1 - r1)
                        r2[pl.ds(row + 128, 8), :] = pack(r0 + j0, r1 + j1)
        def phaseW0():
            for e2 in range(2):
                for h in range(2):
                    if e2 == 0:
                        if h == 1:
                            for g in range(NX0, B * NP): xstart(g)
                            for qh in range(4): w1copy(qh).start()
                        for i in range(K): wcopy(i, h).wait()
                    elif h == 0:
                        for i in range(K): wcopyg(i).wait()
                    for u in range(8): wgroup(e2, h * 8 + u)

        def fblock(b, j):
            tiles = []
            for dt in range(2):
                X = r3[pl.ds((b * 2 + dt) * MP + j * L, N), :]
                top = X[0:64]; bot = X[64:128]
                E = (top & 0xFFFF) | (bot << 16)
                O = lax.shift_right_logical(top, 16) | (bot & jnp.int32(-65536))
                tiles += [bc(E, bf16), bc(O, bf16)]
            Y = jnp.dot(FAr(), jnp.concatenate(tiles, axis=1), preferred_element_type=f32)
            J = b * NJ + j
            for dt in range(2):
                Ye = Y[:, dt * 256:dt * 256 + 128]; Yo = Y[:, dt * 256 + 128:dt * 256 + 256]
                Xf[dt, pl.ds(J * SX, 64), :] = pack(Ye[:64] + Ye[64:], Yo[:64] + Yo[64:])
                Xf[dt, pl.ds(J * SX + 64, 64), :] = pack(Ye[:64], Yo[:64])
                Xf[dt, pl.ds(J * SX + 128, 64), :] = pack(Ye[64:], Yo[64:])
        def phaseF():
            @pl.loop(0, B)
            def _(b):
                for p in range(NP):
                    for dt in range(2): xcopy(b, dt, p).wait()
                    for u in range(JP): fblock(b, p * JP + u)

        def wvpu_pieces(wp, slot):
            e2 = wp // 16; qv = wp % 16
            pb = slot * PS
            out_row = lambda v, k: e2 * (192 * 128) + (v * 64 + k) * 128 + qv * 8
            pieces = []
            def p1(r, pos):
                def run(tok):
                    taps = [r + 8 * a for a in range(4)]
                    words = [wbuf1[e2 * 2 + qv // 8, i, pl.ds(mo((qv % 8) * 8, 8), 8), :] | tok if i < K else None for i in taps]
                    u = [None if wd is None else pltpu.unpack_elementwise(wd, index=pos, packed_dtype=bf16, unpacked_dtype=f32) for wd in words]
                    Pv = pass1(u)
                    for kp in range(8):
                        z = Pv[kp] if r == 0 else cmul(Pv[kp], -2 * np.pi * (kp + 0.5) / N * r)
                        base = pb + ((kp * 2 + pos) * 8 + r) * 16
                        Ps[pl.ds(base, 8), :] = z[0]
                        Ps[pl.ds(base + 8, 8), :] = z[1]
                    s = (u[0] + u[2]) + (u[1] + u[3] if u[3] is not None else u[1])
                    Ps[pl.ds(pb + 2048 + (pos * 8 + r) * 8, 8), :] = s
                return run
            def p2(kp, odd):
                def run(tok):
                    outs = []
                    for pos in range(2):
                        base = pb + ((kp * 2 + pos) * 8) * 16
                        Q = [[Ps[pl.ds(base + r * 16, 8), :], Ps[pl.ds(base + r * 16 + 8, 8), :]] for r in range(8)]
                        for r in TOKR:
                            for h in range(2): Q[r][h] = bc(bc(Q[r][h], i32) | tok, f32)
                        outs.append(p2half(Q, odd, kp))
                    for k in outs[0]:
                        for v in range(3):
                            r3[pl.ds(out_row(v, k), 8), :] = pack(outs[0][k][v], outs[1][k][v])
                return run
            def p3(tok):
                res = []
                for pos in range(2):
                    s = [Ps[pl.ds(pb + 2048 + (pos * 8 + r) * 8, 8), :] for r in range(8)]
                    s[0] = bc(bc(s[0], i32) | tok, f32); s[1] = bc(bc(s[1], i32) | tok, f32)
                    we = (s[0] + s[2]) + (s[4] + s[6]); wo = (s[1] + s[3]) + (s[5] + s[7])
                    res.append((we, wo - we, we - wo))
                for v in range(3):
                    r3[pl.ds(out_row(v, 0), 8), :] = pack(res[0][v], res[1][v])
            for r in range(8):
                for pos in range(2): pieces.append((p1(r, pos), 60 if r == 0 else 108))
            pieces.append((p3, 30))
            for kp in range(8):
                for odd in range(2): pieces.append((p2(kp, odd), 108 if odd else 92))
            return pieces

        def mbin(k, c):
            def lhs(v): return jnp.concatenate([bc(Xf[dt, pl.ds(v * 64 + k, NR, stride=SX), :], bf16) for dt in range(2)], axis=1)
            if c == 0:
                def rhs(v): return jnp.concatenate([bc(r2[pl.ds(e2 * 128 * SW + v * 64 + k, 128, stride=SW), :], bf16) for e2 in range(2)], axis=1)
            else:
                def rhs(v): return jnp.concatenate([bc(r3[pl.ds(mo(e2 * (192 * 128) + (v * 64 + k) * 128, 8), 128), :], bf16) for e2 in range(2)], axis=1)
            k1 = jnp.dot(lhs(0), rhs(0), preferred_element_type=f32)
            k2 = jnp.dot(lhs(1), rhs(1), preferred_element_type=f32)
            k3 = jnp.dot(lhs(2), rhs(2), preferred_element_type=f32)
            Yr = k1 - k3; Yi = k1 + k2
            for e2 in range(2):
                cs = slice(e2 * 128, e2 * 128 + 128)
                Ya[e2, pl.ds(k * SA, 2 * JM), :] = pack(Yr[:2 * JM, cs], Yi[:2 * JM, cs])
                if JH:
                    hi = pack(Yr[2 * JM:, cs], Yi[2 * JM:, cs])
                    if c == 0: Yb[e2, pl.ds(k * SB, 2 * JH), :] = hi
                    else: r2[pl.ds(OC + (e2 * NK + k) * SB, 2 * JH), :] = hi
            return [k1, k2, k3]
        def place(ps, ks, lo, hi, nbins, zm):
            RG = 2 * NR // 8; G = 3 * RG
            tot = float(sum(wt for _, wt in ps)); acc = 0.0
            for p, wt in ps:
                pos = min(int(round(lo + acc / tot * (hi - lo))), nbins * G - 1)
                acc += wt
                d, g = divmod(pos, RG)
                p(bc(ks[d][g * 8:g * 8 + 8, 0:128], i32) & zm)
        def phaseM0():
            RG = 2 * NR // 8; G = 3 * RG
            need = [(8 * q) // WP0 for q in range(4)]
            @pl.loop(0, NI0)
            def _(kk):
                for q in range(4):
                    @pl.when(kk == need[q])
                    def _(): w1copy(q).wait()
                zm = zbuf[...]
                ks = []
                for u in range(UM0): ks += mbin(kk * UM0 + u, 0)
                ps = []
                for u in range(WP0):
                    ps += wvpu_pieces(jnp.minimum(kk * WP0 + u, 31), u % 2)
                place(ps, ks, LAG, UM0 * G - TAIL, UM0, zm)
        SO = L + 4
        NLAST = T - (NJ - 1) * 2 * L
        def vcopy(sp, u, n):
            J = JM + 8 * sp + u
            b = (J >= NJ).astype(i32)
            return mk(v16.at[pl.ds(mo(2 * (8 * sp + u) * SO, 8), n), :],
                      out_hbm.at[b, pl.ds(mo((J - b * NJ) * 2 * L, 8), n), pl.ds(0, 128)], vsem.at[0])
        def vop(sp, op):
            for u in range(8):
                if u == 7 or (JM <= NJ - 1 and u == (NJ - 1 - JM) % 8):
                    J = JM + 8 * sp + u
                    last = jnp.logical_or(J == NJ - 1, J == NR - 1)
                    @pl.when(last)
                    def _(): getattr(vcopy(sp, u, NLAST), op)()
                    @pl.when(jnp.logical_not(last))
                    def _(): getattr(vcopy(sp, u, 2 * L), op)()
                else:
                    getattr(vcopy(sp, u, 2 * L), op)()
        def ivpu_pieces(sp, slot):
            J0 = JM + 8 * sp
            pb = slot * PV
            pieces = []
            def qrow(pos, kp, rho): return pb + ((pos * 8 + kp) * 8 + rho) * 16
            def pA(kp, pos):
                p, e2 = divmod(pos, 2)
                def run(tok):
                    x = []
                    for s_ in range(8):
                        k = kp + 16 * s_
                        kk = k if k < 64 else 127 - k
                        if kk == 0 or kk >= NU:
                            x.append(None); continue
                        wd = Yb[e2, pl.ds(kk * SB + 16 * sp + p, 8, stride=2), :]
                        if s_ < 4: wd = wd | tok
                        re = pltpu.unpack_elementwise(wd, index=0, packed_dtype=bf16, unpacked_dtype=f32)
                        im = pltpu.unpack_elementwise(wd, index=1, packed_dtype=bf16, unpacked_dtype=f32)
                        x.append((re, im))
                    Z = dft8(x)
                    for rho in range(8):
                        z = Z[rho] if rho == 0 else cmul(Z[rho], -2 * np.pi * (kp + 0.5) / N * rho)
                        Ps[pl.ds(qrow(pos, kp, rho), 8), :] = z[0]
                        Ps[pl.ds(qrow(pos, kp, rho) + 8, 8), :] = z[1]
                return run
            held = {}
            def pB(rho, odd, p):
                def run(tok):
                    hv = []
                    for e2 in range(2):
                        pos = p * 2 + e2
                        Q = [[Ps[pl.ds(qrow(pos, kp, rho), 8), :], Ps[pl.ds(qrow(pos, kp, rho) + 8, 8), :]] for kp in range(8)]
                        for kp in range(4):
                            for h in range(2): Q[kp][h] = bc(bc(Q[kp][h], i32) | tok, f32)
                        y = invB(Q, odd)
                        wd = Yb[e2, pl.ds(16 * sp + p, 8, stride=2), :]
                        sp_v = pltpu.unpack_elementwise(wd, index=rho % 2, packed_dtype=bf16, unpacked_dtype=f32)
                        hv.append([v + sp_v for v in y])
                    o = [jnp.tanh(f) * (jnp.tanh(g * 0.5) * 0.5 + 0.5) if 't' not in DBG else f * g for f, g in zip(hv[0], hv[1])]
                    if p == 0: held[0] = o
                    else:
                        for ap in range(6):
                            r = rho + 8 * (2 * ap + odd)
                            vbuf[pl.ds(8 * sp * SO + r, 8, stride=SO), :] = pack(held[0][ap], o[ap])
                return run
            for kp in range(8):
                for pos in range(4): pieces.append((pA(kp, pos), 118))
            for rho in range(8):
                for odd in range(2):
                    for p in range(2): pieces.append((pB(rho, odd, p), (165 if odd else 120) + 60 * p))
            return pieces
        def phaseM1():
            RG = 2 * NR // 8; G = 3 * RG
            @pl.loop(0, NI1)
            def _(kk):
                zm = zbuf[...]
                ks = []
                for u in range(UM1): ks += mbin(kk * UM1 + u, 1)
                ps = []
                for u in range(SP): ps += [q for i_, q in enumerate(ivpu_pieces(kk * SP + u, u % 2)) if not (('A' in DBG and i_ < 32) or ('B' in DBG and i_ >= 32))]
                place(ps, ks, LAG, UM1 * G - TAIL1, UM1, zm)
                if 'd' not in DBG:
                    for u in range(SP): vop(kk * SP + u, 'start')

        def iblock(J):
            tiles = []
            for p in range(2):
                for e2 in range(2):
                    if J < JM: t = Ya[e2, pl.ds(2 * J + p, 64, stride=SA), :]
                    else: t = r2[pl.ds(OC + e2 * NK * SB + 2 * (J - JM) + p, 64, stride=SB), :]
                    tiles.append(bc(t, bf16))
            h = jnp.dot(IAr(), jnp.concatenate(tiles, axis=1), preferred_element_type=f32)
            oe = jnp.tanh(h[:, 0:128]) * (jnp.tanh(h[:, 128:256] * 0.5) * 0.5 + 0.5)
            oo = jnp.tanh(h[:, 256:384]) * (jnp.tanh(h[:, 384:512] * 0.5) * 0.5 + 0.5)
            r2[pl.ds(J * L, L), :] = pack(oe, oo)
        def phaseI(pcs, c):
            for pc in pcs:
                for J in range(pc[0], pc[0] + pc[1]): iblock(J)
                ocp(pc, c).start()

        with scope('W'): phaseW0()
        with scope('F'): phaseF()
        @pl.loop(0, 2)
        def _(c):
            @pl.when(c == 0)
            def _():
                with scope('M0'): phaseM0()
            @pl.when(c == 1)
            def _():
                for e2 in range(2):
                    r2[pl.ds(OC + (e2 * NK + NU) * SB, 2 * JH), :] = zero((2 * JH, 128), i32)
                with scope('M1'): phaseM1()
                for pc in PCA: ocp(pc, 0).wait()
            with scope('IA'): phaseI(PCA, c)
        with scope('IC'): phaseI(PCC, 1)
        with scope('end'):
            if 'd' not in DBG:
                @pl.loop(0, NSP)
                def _(h): vop(h, 'wait')
            for pc in PCA + PCC: ocp(pc, 1).wait()

    cst = consts(K)
    def f(x, w):
        return pl.pallas_call(kernel,
            out_shape=jax.ShapeDtypeStruct((B, T, D), bf16),
            in_specs=[pl.BlockSpec(memory_space=pl.ANY)] * 3,
            out_specs=pl.BlockSpec(memory_space=pl.ANY),
            scratch_shapes=[pltpu.VMEM(cst.shape, i32), pltpu.VMEM((2, 32 * SI, 128), i32), pltpu.VMEM((4, K, 64, 128), i32),
                            pltpu.VMEM((2, NR * SX, 128), i32), pltpu.VMEM((R2, 128), i32), pltpu.VMEM((R3, 128), i32),
                            pltpu.VMEM((2, NK * SA, 128), i32), pltpu.VMEM((2, NK * SB, 128), i32), pltpu.VMEM((max(JH, 8) * (L + 4), 128), i32), pltpu.VMEM((2 * PV, 128), f32), pltpu.VMEM((8, 128), i32),
                            pltpu.SemaphoreType.DMA((1,)), pltpu.SemaphoreType.DMA((B * 2, NP)), pltpu.SemaphoreType.DMA((3,)),
                            pltpu.SemaphoreType.DMA((len(PCA) + len(PCC),)), pltpu.SemaphoreType.DMA((4,)),
                            pltpu.SemaphoreType.DMA((1,))],
            compiler_params=pltpu.CompilerParams(vmem_limit_bytes=127 * 1024 * 1024, flags=flags),
        )(x, w, jnp.asarray(cst))
    return f


@jax.jit
def pallas_standalone__autoregressive_conv_wavernn__speech_kernel(x: jax.Array, w: jax.Array):
    B, T, D = x.shape
    K = w.shape[0]
    return make(B, T, D, K, scopes=False)(x, w)
```

```python
import contextlib
import numpy as np
import jax, jax.numpy as jnp
from jax import lax
from jax.experimental import pallas as pl
from jax.experimental.pallas import tpu as pltpu
import ml_dtypes

N = 128
L = 96
NK = 64
NU = 63
SX = 196; SW = 196; SI = 132; SY = 340


def _pack_rows(a):
    u = a.astype(np.float32).astype(ml_dtypes.bfloat16).view(np.uint16).astype(np.uint32)
    return (u[0::2] | (u[1::2] << 16)).view(np.int32)


def consts(K):
    m = L + K - 1
    assert m == 2 * (NU - 1) + 2
    th = 2 * np.pi * (np.arange(NK) + 0.5) / N
    ks = np.arange(1, NU)
    z = np.concatenate([np.exp(-1j * th[ks]), np.exp(1j * th[ks]), [1.0, -1.0]])
    V = z[:, None] ** np.arange(m)[None]
    BT = np.linalg.inv(V).T
    off = 32 - (K - 1)
    F = np.zeros((128, N))
    F[ks, off:off + m] = 2 * BT[:NU - 1].real
    F[64 + ks, off:off + m] = 2 * BT[:NU - 1].imag
    bp, bm = BT[-2].real, BT[-1].real
    F[0, off:off + m] = bp + bm
    F[64, off:off + m] = bp - bm
    Fp = np.zeros_like(F); Fp[:, 0::2] = F[:, :64]; Fp[:, 1::2] = F[:, 64:]
    i = np.arange(32)
    Gc = np.cos(th[:, None] * i[None]); Gs = -np.sin(th[:, None] * i[None])
    Gc[0] = (i % 2 == 0); Gs[0] = (i % 2 == 1)
    Gc[NU:] = 0; Gs[NU:] = 0
    Gc[:, K:] = 0; Gs[:, K:] = 0
    GW = np.zeros((512, 128))
    for qs in range(2):
        for kg in range(8):
            base = qs * 256 + kg * 32
            for h, (G, dpar) in enumerate([(Gc, 0), (Gc, 1), (Gs, 0), (Gs, 1)]):
                GW[base + h * 8:base + h * 8 + 8, 2 * (qs * 32 + i) + dpar] = G[kg * 8:kg * 8 + 8, :]
    r = np.arange(L)
    IA = np.zeros((L, 128))
    IA[:, 0::2] = np.cos(r[:, None] * th[None]); IA[:, 1::2] = np.sin(r[:, None] * th[None])
    IA[:, 0] = (1 + (-1.0) ** r) / 2; IA[:, 1] = (1 - (-1.0) ** r) / 2
    IA[:, 2 * NU:] = 0
    sgn = np.ones((8, 128), np.float32); sgn[0] = -1
    return np.concatenate([_pack_rows(GW), _pack_rows(Fp), _pack_rows(IA), sgn.view(np.int32)], 0)


def f32c(v): return float(np.float32(v))
def pass1(u):
    out = [None] * 8
    for kp in range(4):
        ph = 2 * np.pi * (kp + 0.5) / 16
        c1, s1 = np.cos(ph), -np.sin(ph); c2, s2 = np.cos(2 * ph), -np.sin(2 * ph); c3, s3 = np.cos(3 * ph), -np.sin(3 * ph)
        Er = u[0] + u[2] * f32c(c2); Ei = u[2] * f32c(s2)
        if u[3] is not None:
            Or = u[1] * f32c(c1) + u[3] * f32c(c3); Oi = u[1] * f32c(s1) + u[3] * f32c(s3)
        else:
            Or = u[1] * f32c(c1); Oi = u[1] * f32c(s1)
        out[kp] = (Er + Or, Ei + Oi)
        out[7 - kp] = (Er - Or, Oi - Ei)
    return out
def cmul(z, ang, sc=1.0):
    c, s = f32c(sc * np.cos(ang)), f32c(sc * np.sin(ang))
    return (z[0] * c - z[1] * s, z[0] * s + z[1] * c)
def p2half(Q, odd, kp):
    def half(x):
        if not odd:
            a = (x[0][0] + x[2][0], x[0][1] + x[2][1]); c = (x[1][0] + x[3][0], x[1][1] + x[3][1])
            return {0: (a[0] + c[0], a[1] + c[1]), 2: (a[0] - c[0], a[1] - c[1])}
        b = (x[0][0] - x[2][0], x[0][1] - x[2][1]); d = (x[1][0] - x[3][0], x[1][1] - x[3][1])
        return {1: (b[0] + d[1], b[1] - d[0]), 3: (b[0] - d[1], b[1] + d[0])}
    A = half([Q[0], Q[2], Q[4], Q[6]]); Bv = half([Q[1], Q[3], Q[5], Q[7]])
    h = f32c(np.sqrt(0.5)); o = {}
    for s in A:
        Ar, Ai = A[s]; br, bi = Bv[s]
        k = kp + 16 * s; km = 127 - kp - 16 * (s + 4)
        if s == 0:   Br, Bi, nBi = br, bi, None
        elif s == 1: Br, Bi, nBi = (br + bi) * h, (bi - br) * h, None
        elif s == 2: Br, Bi, nBi = bi, None, br
        else:        Br, Bi, nBi = (bi - br) * h, None, (br + bi) * h
        if 0 < k < NU:
            Re = Ar + Br
            Im = Ai + Bi if nBi is None else Ai - nBi
            o[k] = (Re, Im - Re, Re + Im)
        if 0 < km < NU:
            Re2 = Ar - Br
            if nBi is None:
                nIm2 = Bi - Ai
                o[km] = (Re2, nIm2 - Re2, Re2 + nIm2)
            else:
                pIm2 = nBi + Ai
                o[km] = (Re2, -(pIm2 + Re2), Re2 - pIm2)
    return o

def _add(a, b): return b if a is None else (a if b is None else a + b)
def _sub(a, b): return a if b is None else (-b if a is None else a - b)
def cadd(x, y):
    if x is None: return y
    if y is None: return x
    return (x[0] + y[0], x[1] + y[1])
def csub(x, y):
    if y is None: return x
    if x is None: return (-y[0], -y[1])
    return (x[0] - y[0], x[1] - y[1])
def dft4c(x0, x1, y2, y3):
    c = (x1[0] + y3[0], x1[1] - y3[1]); d = (x1[0] - y3[0], x1[1] + y3[1])
    if x0 is None:
        assert y2 is None
        return [c, (d[1], -d[0]), (-c[0], -c[1]), (-d[1], d[0])]
    a = (x0[0] + y2[0], x0[1] - y2[1]); b = (x0[0] - y2[0], x0[1] + y2[1])
    return [(a[0] + c[0], a[1] + c[1]), (b[0] + d[1], b[1] - d[0]), (a[0] - c[0], a[1] - c[1]), (b[0] - d[1], b[1] + d[0])]
def dft8(x):
    A = dft4c(x[0], x[2], x[4], x[6]); Bv = dft4c(x[1], x[3], x[5], x[7])
    h = f32c(np.sqrt(0.5))
    b0, b1, b2, b3 = Bv
    t1 = ((b1[0] + b1[1]) * h, (b1[1] - b1[0]) * h)
    out = [None] * 8
    out[0] = (A[0][0] + b0[0], A[0][1] + b0[1]); out[4] = (A[0][0] - b0[0], A[0][1] - b0[1])
    out[1] = (A[1][0] + t1[0], A[1][1] + t1[1]); out[5] = (A[1][0] - t1[0], A[1][1] - t1[1])
    out[2] = (A[2][0] + b2[1], A[2][1] - b2[0]); out[6] = (A[2][0] - b2[1], A[2][1] + b2[0])
    u3 = (b3[1] - b3[0]) * h; v3 = (b3[0] + b3[1]) * h
    out[3] = (A[3][0] + u3, A[3][1] - v3); out[7] = (A[3][0] - u3, A[3][1] + v3)
    return out
def inv6(P):
    h = f32c(np.sqrt(0.5)); y = [None] * 6
    for par in range(2):
        R = []
        for k in range(2):
            x, z = P[k], P[3 - k]
            if par == 0: v = (x[0] + z[0], x[1] - z[1])
            else:
                v = (x[0] - z[0], x[1] + z[1]); v = cmul(v, -2 * np.pi * (k + 0.5) / 8)
            R.append(v)
        (r0, i0), (r1, i1) = R
        y[par] = r0 + r1
        y[par + 2] = ((r0 + i0) + (i1 - r1)) * h
        y[par + 4] = i0 - i1
    return y
def invB(Q, odd):
    P = []
    for k in range(4):
        x, z = Q[k], Q[7 - k]
        if not odd: P.append((x[0] + z[0], x[1] - z[1]))
        else: P.append(cmul((x[0] - z[0], x[1] + z[1]), -2 * np.pi * (k + 0.5) / 16))
    return inv6(P)


def make(B, T, D, K, UI=14, NI0=7, NI1=7, SP=2, scopes=True, flags=None, TOKR=(0, 1, 2, 3), NP=6, NX0=2, LAG=0, TAIL=8, TAIL1=40, DBG='', TH0=(0, 1), TH1=(0, 1), FOLD=True, TKB=4, TKA=4, FINE=True):
    M = T // 2; NJ = -(-M // L); MP = (NJ - 1) * L + N; NR = B * NJ
    f32 = jnp.float32; bf16 = jnp.bfloat16; i32 = jnp.int32
    JP = NJ // NP; TP = JP * 2 * L; TL = T - (NP - 1) * TP
    UM0 = NU // NI0; WP0 = -(-32 // NI0)
    UM1 = NU // NI1; NSP = NI1 * SP; JM = NR - 8 * NSP
    assert 0 < JM <= NR and JM % 4 == 0
    JH = NR - JM
    def odd4(n): return n + 4 if n % 8 == 0 else n
    SA = odd4(2 * JM); SB = odd4(2 * JH)
    def pieces_of(J0, J1, sem0):
        out = []; J = J0
        while J < J1:
            n = min(UI, J1 - J, NJ - J % NJ); out.append((J, n, sem0 + len(out))); J += n
        return out
    PCA = pieces_of(0, JM, 0); PCC = pieces_of(JM, NR, len(PCA))
    assert NJ % NP == 0 and NJ % UI == 0 and NU % NI0 == 0 and NU % UM1 == 0
    def bc(x, t): return pltpu.bitcast(x, t)
    def pack(a, b): return pltpu.pack_elementwise([a, b], packed_dtype=bf16)
    scope = jax.named_scope if scopes else (lambda n: contextlib.nullcontext())
    R3 = 2 * 192 * 128
    R2 = 2 * 128 * SW
    assert 4 * MP <= R3 and B * NJ * L <= R2
    H2 = D // 2
    PS = 2048 + 128; PV = 4096
    OC = B * NJ * L
    assert OC + 2 * NK * SB <= R2
    NO = NJ // UI

    def kernel(x_hbm, w_hbm, c_hbm, out_hbm,
               cbuf, wbuf, wbuf1, Xf, r2, r3, Ya, Yb, vbuf, Ps, zbuf, csem, xsem, wsem, osem, w1sem, vsem):
        x16 = r3.bitcast(bf16); wb16 = wbuf.bitcast(bf16); w116 = wbuf1.bitcast(bf16); o16 = r2.bitcast(bf16); v16 = vbuf.bitcast(bf16)
        mk = pltpu.make_async_copy
        mo = pl.multiple_of
        ccopy = mk(c_hbm, cbuf, csem.at[0])
        def wcopy(i, h):
            return mk(w_hbm.at[i, pl.ds(mo(h * H2, 8), H2), pl.ds(0, 128)],
                      wb16.at[0, pl.ds(mo(i * (2 * SI) + h * H2, 8), H2), :], wsem.at[h])
        def wcopyg(i):
            return mk(w_hbm.at[i, :, pl.ds(D, 128)], wb16.at[1, pl.ds(mo(i * (2 * SI), 8), D), :], wsem.at[2])
        def w1copy(qh):
            e2 = qh // 2; h = qh % 2
            return mk(w_hbm.at[:, pl.ds(mo(h * H2, 8), H2), pl.ds(mo((1 + 2 * e2) * 128, 128), 128)], w116.at[qh], w1sem.at[qh])
        def xcopy(b, dt, p):
            n = TP if p < NP - 1 else TL
            row0 = mo((b * 2 + dt) * (2 * MP) + 64 + p * TP, 8)
            return mk(x_hbm.at[b, pl.ds(p * TP, n), pl.ds(dt * 128, 128)], x16.at[pl.ds(row0, n), :], xsem.at[b * 2 + dt, p])
        def xstart(g):
            b, p = divmod(g, NP)
            for dt in range(2): xcopy(b, dt, p).start()
        def ocp(pc, c):
            J, nb, si = pc; b, j = divmod(J, NJ)
            t0 = j * 2 * L; n = min(T, (j + nb) * 2 * L) - t0
            return mk(o16.at[pl.ds(J * 2 * L, n), :], out_hbm.at[b, pl.ds(t0, n), pl.ds(mo(c * 128, 128), 128)], osem.at[si])

        @pl.loop(0, K)
        def _(i): wcopy(i, 0).start()
        ccopy.start()
        @pl.loop(0, K)
        def _(i): wcopy(i, 1).start()
        @pl.loop(0, K)
        def _(i): wcopyg(i).start()
        for g in range(NX0): xstart(g)
        zero = jnp.zeros
        for s in range(B * 2):
            r3[pl.ds(s * MP, 32), :] = zero((32, 128), i32)
            r3[pl.ds(s * MP + 32 + M, MP - 32 - M), :] = zero((MP - 32 - M, 128), i32)
        for e2 in range(2):
            wbuf[e2, pl.ds(K * SI, (32 - K) * SI), :] = zero(((32 - K) * SI, 128), i32)
            Ya[e2, pl.ds(NU * SA, 2 * JM), :] = zero((2 * JM, 128), i32)
        zbuf[...] = zero((8, 128), i32)
        ccopy.wait()
        GWr = lambda: bc(cbuf[0:256, :], bf16)
        FAr = lambda: bc(cbuf[256:320, :], bf16)
        IAr = lambda: bc(cbuf[320:368, :], bf16)
        SGN = lambda: bc(cbuf[368:376, :], f32)

        def wgroup(e2, g):
            tiles = []
            for qp in range(4):
                q0 = g * 8 + qp * 2
                t = jnp.concatenate([wbuf[e2, pl.ds(q0, 32, stride=SI), :], wbuf[e2, pl.ds(q0 + 1, 32, stride=SI), :]], axis=0)
                tiles.append(bc(t, bf16))
            o = jnp.dot(GWr(), jnp.concatenate(tiles, axis=1), preferred_element_type=f32)
            sg = SGN()
            for qp in range(4):
                col = qp * 128
                for qs in range(2):
                    q = g * 8 + qp * 2 + qs
                    for kg in range(8):
                        base = qs * 256 + kg * 32
                        r0 = o[base:base + 8, col:col + 128]; r1 = o[base + 8:base + 16, col:col + 128]
                        i0 = o[base + 16:base + 24, col:col + 128]; i1 = o[base + 24:base + 32, col:col + 128]
                        j0, j1 = (i0 * sg, i1 * sg) if kg == 0 else (i0, i1)
                        row = e2 * 128 * SW + q * SW + kg * 8
                        r2[pl.ds(row, 8), :] = pack(r0, r1)
                        r2[pl.ds(row + 64, 8), :] = pack(i0 - r0, i1 - r1)
                        r2[pl.ds(row + 128, 8), :] = pack(r0 + j0, r1 + j1)
        def phaseW0():
            for e2 in range(2):
                for h in range(2):
                    if e2 == 0:
                        if h == 1:
                            for g in range(NX0, B * NP): xstart(g)
                            for qh in range(4): w1copy(qh).start()
                        for i in range(K): wcopy(i, h).wait()
                    elif h == 0:
                        for i in range(K): wcopyg(i).wait()
                    for u in range(8): wgroup(e2, h * 8 + u)

        def fblock(b, j):
            tiles = []
            for dt in range(2):
                X = r3[pl.ds((b * 2 + dt) * MP + j * L, N), :]
                top = X[0:64]; bot = X[64:128]
                E = (top & 0xFFFF) | (bot << 16)
                O = lax.shift_right_logical(top, 16) | (bot & jnp.int32(-65536))
                tiles += [bc(E, bf16), bc(O, bf16)]
            Y = jnp.dot(FAr(), jnp.concatenate(tiles, axis=1), preferred_element_type=f32)
            J = b * NJ + j
            for dt in range(2):
                Ye = Y[:, dt * 256:dt * 256 + 128]; Yo = Y[:, dt * 256 + 128:dt * 256 + 256]
                Xf[dt, pl.ds(J * SX, 64), :] = pack(Ye[:64] + Ye[64:], Yo[:64] + Yo[64:])
                Xf[dt, pl.ds(J * SX + 64, 64), :] = pack(Ye[:64], Yo[:64])
                Xf[dt, pl.ds(J * SX + 128, 64), :] = pack(Ye[64:], Yo[64:])
        def phaseF():
            @pl.loop(0, B)
            def _(b):
                for p in range(NP):
                    for dt in range(2): xcopy(b, dt, p).wait()
                    for u in range(JP): fblock(b, p * JP + u)

        def wvpu_pieces(wp, slot):
            e2 = wp // 16; qv = wp % 16
            pb = slot * PS
            out_row = lambda v, k: e2 * (192 * 128) + (v * 64 + k) * 128 + qv * 8
            pieces = []
            def p1(r, pos):
                def run(tok):
                    taps = [r + 8 * a for a in range(4)]
                    words = [wbuf1[e2 * 2 + qv // 8, i, pl.ds(mo((qv % 8) * 8, 8), 8), :] | tok if i < K else None for i in taps]
                    u = [None if wd is None else pltpu.unpack_elementwise(wd, index=pos, packed_dtype=bf16, unpacked_dtype=f32) for wd in words]
                    Pv = pass1(u)
                    for kp in range(8):
                        z = Pv[kp] if r == 0 else cmul(Pv[kp], -2 * np.pi * (kp + 0.5) / N * r)
                        base = pb + ((kp * 2 + pos) * 8 + r) * 16
                        Ps[pl.ds(base, 8), :] = z[0]
                        Ps[pl.ds(base + 8, 8), :] = z[1]
                    s = (u[0] + u[2]) + (u[1] + u[3] if u[3] is not None else u[1])
                    Ps[pl.ds(pb + 2048 + (pos * 8 + r) * 8, 8), :] = s
                return run
            def p2(kp, odd):
                def run(tok):
                    outs = []
                    for pos in range(2):
                        base = pb + ((kp * 2 + pos) * 8) * 16
                        Q = [[Ps[pl.ds(base + r * 16, 8), :], Ps[pl.ds(base + r * 16 + 8, 8), :]] for r in range(8)]
                        for r in TOKR:
                            for h in TH0: Q[r][h] = bc(bc(Q[r][h], i32) | tok, f32)
                        outs.append(p2half(Q, odd, kp))
                    for k in outs[0]:
                        for v in range(3):
                            r3[pl.ds(out_row(v, k), 8), :] = pack(outs[0][k][v], outs[1][k][v])
                return run
            def p3(tok):
                res = []
                for pos in range(2):
                    s = [Ps[pl.ds(pb + 2048 + (pos * 8 + r) * 8, 8), :] for r in range(8)]
                    s[0] = bc(bc(s[0], i32) | tok, f32); s[1] = bc(bc(s[1], i32) | tok, f32)
                    we = (s[0] + s[2]) + (s[4] + s[6]); wo = (s[1] + s[3]) + (s[5] + s[7])
                    res.append((we, wo - we, we - wo))
                for v in range(3):
                    r3[pl.ds(out_row(v, 0), 8), :] = pack(res[0][v], res[1][v])
            for r in range(8):
                for pos in range(2): pieces.append((p1(r, pos), 60 if r == 0 else 108))
            pieces.append((p3, 30))
            for kp in range(8):
                for odd in range(2): pieces.append((p2(kp, odd), 108 if odd else 92))
            return pieces

        def mbin(k, c):
            def lhs(v): return jnp.concatenate([bc(Xf[dt, pl.ds(v * 64 + k, NR, stride=SX), :], bf16) for dt in range(2)], axis=1)
            if c == 0:
                def rhs(v): return jnp.concatenate([bc(r2[pl.ds(e2 * 128 * SW + v * 64 + k, 128, stride=SW), :], bf16) for e2 in range(2)], axis=1)
            else:
                def rhs(v): return jnp.concatenate([bc(r3[pl.ds(mo(e2 * (192 * 128) + (v * 64 + k) * 128, 8), 128), :], bf16) for e2 in range(2)], axis=1)
            k1 = jnp.dot(lhs(0), rhs(0), preferred_element_type=f32)
            k2 = jnp.dot(lhs(1), rhs(1), preferred_element_type=f32)
            k3 = jnp.dot(lhs(2), rhs(2), preferred_element_type=f32)
            Yr = k1 - k3; Yi = k1 + k2
            for e2 in range(2):
                cs = slice(e2 * 128, e2 * 128 + 128)
                Ya[e2, pl.ds(k * SA, 2 * JM), :] = pack(Yr[:2 * JM, cs], Yi[:2 * JM, cs])
                if JH:
                    hi = pack(Yr[2 * JM:, cs], Yi[2 * JM:, cs])
                    if c == 0: Yb[e2, pl.ds(k * SB, 2 * JH), :] = hi
                    else: r2[pl.ds(OC + (e2 * NK + k) * SB, 2 * JH), :] = hi
            return [k1, k2, k3]
        def place(ps, ks, lo, hi, nbins, zm):
            RG = 2 * NR // 8; G = 3 * RG
            tot = float(sum(wt for _, wt in ps)); acc = 0.0
            for p, wt in ps:
                pos = min(int(round(lo + acc / tot * (hi - lo))), nbins * G - 1)
                acc += wt
                d, g = divmod(pos, RG)
                p(bc(ks[d][g * 8:g * 8 + 8, 0:128], i32) & zm)
        def phaseM0():
            RG = 2 * NR // 8; G = 3 * RG
            need = [(8 * q) // WP0 for q in range(4)]
            @pl.loop(0, NI0)
            def _(kk):
                for q in range(4):
                    @pl.when(kk == need[q])
                    def _(): w1copy(q).wait()
                zm = zbuf[...]
                ks = []
                for u in range(UM0): ks += mbin(kk * UM0 + u, 0)
                ps = []
                for u in range(WP0):
                    ps += wvpu_pieces(jnp.minimum(kk * WP0 + u, 31), u % 2)
                place(ps, ks, LAG, UM0 * G - TAIL, UM0, zm)
        SO = L + 4
        NLAST = T - (NJ - 1) * 2 * L
        def vcopy(sp, u, n):
            J = JM + 8 * sp + u
            b = (J >= NJ).astype(i32)
            return mk(v16.at[pl.ds(mo(2 * (8 * sp + u) * SO, 8), n), :],
                      out_hbm.at[b, pl.ds(mo((J - b * NJ) * 2 * L, 8), n), pl.ds(0, 128)], vsem.at[0])
        def vop(sp, op):
            for u in range(8):
                if u == 7 or (JM <= NJ - 1 and u == (NJ - 1 - JM) % 8):
                    J = JM + 8 * sp + u
                    last = jnp.logical_or(J == NJ - 1, J == NR - 1)
                    @pl.when(last)
                    def _(): getattr(vcopy(sp, u, NLAST), op)()
                    @pl.when(jnp.logical_not(last))
                    def _(): getattr(vcopy(sp, u, 2 * L), op)()
                else:
                    getattr(vcopy(sp, u, 2 * L), op)()
        def ivpu_pieces(sp, slot):
            J0 = JM + 8 * sp
            pb = slot * PV
            pieces = []
            def qrow(pos, kp, rho): return pb + ((pos * 8 + kp) * 8 + rho) * 16
            def pA(kp, pos):
                p, e2 = divmod(pos, 2)
                def run(tok):
                    x = []
                    for s_ in range(8):
                        k = kp + 16 * s_
                        kk = k if k < 64 else 127 - k
                        if kk == 0 or kk >= NU:
                            x.append(None); continue
                        wd = Yb[e2, pl.ds(kk * SB + 16 * sp + p, 8, stride=2), :]
                        if s_ < TKA: wd = wd | tok
                        re = pltpu.unpack_elementwise(wd, index=0, packed_dtype=bf16, unpacked_dtype=f32)
                        im = pltpu.unpack_elementwise(wd, index=1, packed_dtype=bf16, unpacked_dtype=f32)
                        x.append((re, im))
                    Z = dft8(x)
                    for rho in range(8):
                        sc = 0.5 if (FOLD and e2 == 1) else 1.0
                        if rho == 0: z = Z[0] if sc == 1.0 else (Z[0][0] * sc, Z[0][1] * sc)
                        else: z = cmul(Z[rho], -2 * np.pi * (kp + 0.5) / N * rho, sc)
                        Ps[pl.ds(qrow(pos, kp, rho), 8), :] = z[0]
                        Ps[pl.ds(qrow(pos, kp, rho) + 8, 8), :] = z[1]
                return run
            held = {}
            def pBpos(rho, odd, p, e2, tok):
                pos = p * 2 + e2
                Q = [[Ps[pl.ds(qrow(pos, kp, rho), 8), :], Ps[pl.ds(qrow(pos, kp, rho) + 8, 8), :]] for kp in range(8)]
                for kp in range(TKB):
                    for h in TH1: Q[kp][h] = bc(bc(Q[kp][h], i32) | tok, f32)
                y = invB(Q, odd)
                wd = Yb[e2, pl.ds(16 * sp + p, 8, stride=2), :]
                sp_v = pltpu.unpack_elementwise(wd, index=rho % 2, packed_dtype=bf16, unpacked_dtype=f32)
                if FOLD and e2 == 1: sp_v = sp_v * 0.5
                h = [v + sp_v for v in y]
                if e2 == 0:
                    held['f'] = [jnp.tanh(v) for v in h]
                    return
                o = [f * (jnp.tanh(g if FOLD else g * 0.5) * 0.5 + 0.5) for f, g in zip(held['f'], h)]
                if p == 0: held[0] = o
                else:
                    for ap in range(6):
                        r = rho + 8 * (2 * ap + odd)
                        vbuf[pl.ds(8 * sp * SO + r, 8, stride=SO), :] = pack(held[0][ap], o[ap])
            def pB(rho, odd, p, e2s):
                def run(tok):
                    for e2 in e2s: pBpos(rho, odd, p, e2, tok)
                return run
            for kp in range(8):
                for pos in range(4): pieces.append((pA(kp, pos), 118))
            for rho in range(8):
                for odd in range(2):
                    for p in range(2):
                        if FINE:
                            pieces.append((pB(rho, odd, p, (0,)), (86 if odd else 62)))
                            pieces.append((pB(rho, odd, p, (1,)), (105 if odd else 81) + 6 * p))
                        else: pieces.append((pB(rho, odd, p, (0, 1)), (190 if odd else 143) + 6 * p))
            return pieces
        def phaseM1():
            RG = 2 * NR // 8; G = 3 * RG
            @pl.loop(0, NI1)
            def _(kk):
                zm = zbuf[...]
                ks = []
                for u in range(UM1): ks += mbin(kk * UM1 + u, 1)
                ps = []
                for u in range(SP): ps += [q for i_, q in enumerate(ivpu_pieces(kk * SP + u, u % 2)) if not (('A' in DBG and i_ < 32) or ('B' in DBG and i_ >= 32))]
                place(ps, ks, LAG, UM1 * G - TAIL1, UM1, zm)
                if 'd' not in DBG:
                    for u in range(SP): vop(kk * SP + u, 'start')

        def iblock(J):
            tiles = []
            for p in range(2):
                for e2 in range(2):
                    if J < JM: t = Ya[e2, pl.ds(2 * J + p, 64, stride=SA), :]
                    else: t = r2[pl.ds(OC + e2 * NK * SB + 2 * (J - JM) + p, 64, stride=SB), :]
                    tiles.append(bc(t, bf16))
            h = jnp.dot(IAr(), jnp.concatenate(tiles, axis=1), preferred_element_type=f32)
            oe = jnp.tanh(h[:, 0:128]) * (jnp.tanh(h[:, 128:256] * 0.5) * 0.5 + 0.5)
            oo = jnp.tanh(h[:, 256:384]) * (jnp.tanh(h[:, 384:512] * 0.5) * 0.5 + 0.5)
            r2[pl.ds(J * L, L), :] = pack(oe, oo)
        def phaseI(pcs, c):
            for pc in pcs:
                for J in range(pc[0], pc[0] + pc[1]): iblock(J)
                ocp(pc, c).start()

        with scope('W'): phaseW0()
        with scope('F'): phaseF()
        @pl.loop(0, 2)
        def _(c):
            @pl.when(c == 0)
            def _():
                with scope('M0'): phaseM0()
            @pl.when(c == 1)
            def _():
                for e2 in range(2):
                    r2[pl.ds(OC + (e2 * NK + NU) * SB, 2 * JH), :] = zero((2 * JH, 128), i32)
                with scope('M1'): phaseM1()
                for pc in PCA: ocp(pc, 0).wait()
            with scope('IA'): phaseI(PCA, c)
        with scope('IC'): phaseI(PCC, 1)
        with scope('end'):
            if 'd' not in DBG:
                @pl.loop(0, NSP)
                def _(h): vop(h, 'wait')
            for pc in PCA + PCC: ocp(pc, 1).wait()

    cst = consts(K)
    def f(x, w):
        return pl.pallas_call(kernel,
            out_shape=jax.ShapeDtypeStruct((B, T, D), bf16),
            in_specs=[pl.BlockSpec(memory_space=pl.ANY)] * 3,
            out_specs=pl.BlockSpec(memory_space=pl.ANY),
            scratch_shapes=[pltpu.VMEM(cst.shape, i32), pltpu.VMEM((2, 32 * SI, 128), i32), pltpu.VMEM((4, K, 64, 128), i32),
                            pltpu.VMEM((2, NR * SX, 128), i32), pltpu.VMEM((R2, 128), i32), pltpu.VMEM((R3, 128), i32),
                            pltpu.VMEM((2, NK * SA, 128), i32), pltpu.VMEM((2, NK * SB, 128), i32), pltpu.VMEM((max(JH, 8) * (L + 4), 128), i32), pltpu.VMEM((2 * PV, 128), f32), pltpu.VMEM((8, 128), i32),
                            pltpu.SemaphoreType.DMA((1,)), pltpu.SemaphoreType.DMA((B * 2, NP)), pltpu.SemaphoreType.DMA((3,)),
                            pltpu.SemaphoreType.DMA((len(PCA) + len(PCC),)), pltpu.SemaphoreType.DMA((4,)),
                            pltpu.SemaphoreType.DMA((1,))],
            compiler_params=pltpu.CompilerParams(vmem_limit_bytes=127 * 1024 * 1024, flags=flags),
        )(x, w, jnp.asarray(cst))
    return f


@jax.jit
def pallas_standalone__autoregressive_conv_wavernn__speech_kernel(x: jax.Array, w: jax.Array):
    B, T, D = x.shape
    K = w.shape[0]
    return make(B, T, D, K, scopes=False)(x, w)
```

```python
import contextlib
import numpy as np
import jax, jax.numpy as jnp
from jax import lax
from jax.experimental import pallas as pl
from jax.experimental.pallas import tpu as pltpu
import ml_dtypes

N = 128
L = 96
NK = 64
NU = 63
SX = 196; SW = 196; SI = 132; SY = 340


def _pack_rows(a):
    u = a.astype(np.float32).astype(ml_dtypes.bfloat16).view(np.uint16).astype(np.uint32)
    return (u[0::2] | (u[1::2] << 16)).view(np.int32)


def consts(K):
    m = L + K - 1
    assert m == 2 * (NU - 1) + 2
    th = 2 * np.pi * (np.arange(NK) + 0.5) / N
    ks = np.arange(1, NU)
    z = np.concatenate([np.exp(-1j * th[ks]), np.exp(1j * th[ks]), [1.0, -1.0]])
    V = z[:, None] ** np.arange(m)[None]
    BT = np.linalg.inv(V).T
    off = 32 - (K - 1)
    F = np.zeros((128, N))
    F[ks, off:off + m] = 2 * BT[:NU - 1].real
    F[64 + ks, off:off + m] = 2 * BT[:NU - 1].imag
    bp, bm = BT[-2].real, BT[-1].real
    F[0, off:off + m] = bp + bm
    F[64, off:off + m] = bp - bm
    Fp = np.zeros_like(F); Fp[:, 0::2] = F[:, :64]; Fp[:, 1::2] = F[:, 64:]
    i = np.arange(32)
    Gc = np.cos(th[:, None] * i[None]); Gs = -np.sin(th[:, None] * i[None])
    Gc[0] = (i % 2 == 0); Gs[0] = (i % 2 == 1)
    Gc[NU:] = 0; Gs[NU:] = 0
    Gc[:, K:] = 0; Gs[:, K:] = 0
    GW = np.zeros((512, 128))
    for qs in range(2):
        for kg in range(8):
            base = qs * 256 + kg * 32
            for h, (G, dpar) in enumerate([(Gc, 0), (Gc, 1), (Gs, 0), (Gs, 1)]):
                GW[base + h * 8:base + h * 8 + 8, 2 * (qs * 32 + i) + dpar] = G[kg * 8:kg * 8 + 8, :]
    r = np.arange(L)
    IA = np.zeros((L, 128))
    IA[:, 0::2] = np.cos(r[:, None] * th[None]); IA[:, 1::2] = np.sin(r[:, None] * th[None])
    IA[:, 0] = (1 + (-1.0) ** r) / 2; IA[:, 1] = (1 - (-1.0) ** r) / 2
    IA[:, 2 * NU:] = 0
    sgn = np.ones((8, 128), np.float32); sgn[0] = -1
    return np.concatenate([_pack_rows(GW), _pack_rows(Fp), _pack_rows(IA), sgn.view(np.int32)], 0)


def f32c(v): return float(np.float32(v))
def pass1(u):
    out = [None] * 8
    for kp in range(4):
        ph = 2 * np.pi * (kp + 0.5) / 16
        c1, s1 = np.cos(ph), -np.sin(ph); c2, s2 = np.cos(2 * ph), -np.sin(2 * ph); c3, s3 = np.cos(3 * ph), -np.sin(3 * ph)
        Er = u[0] + u[2] * f32c(c2); Ei = u[2] * f32c(s2)
        if u[3] is not None:
            Or = u[1] * f32c(c1) + u[3] * f32c(c3); Oi = u[1] * f32c(s1) + u[3] * f32c(s3)
        else:
            Or = u[1] * f32c(c1); Oi = u[1] * f32c(s1)
        out[kp] = (Er + Or, Ei + Oi)
        out[7 - kp] = (Er - Or, Oi - Ei)
    return out
def cmul(z, ang, sc=1.0):
    c, s = f32c(sc * np.cos(ang)), f32c(sc * np.sin(ang))
    return (z[0] * c - z[1] * s, z[0] * s + z[1] * c)
def p2half(Q, odd, kp):
    def half(x):
        if not odd:
            a = (x[0][0] + x[2][0], x[0][1] + x[2][1]); c = (x[1][0] + x[3][0], x[1][1] + x[3][1])
            return {0: (a[0] + c[0], a[1] + c[1]), 2: (a[0] - c[0], a[1] - c[1])}
        b = (x[0][0] - x[2][0], x[0][1] - x[2][1]); d = (x[1][0] - x[3][0], x[1][1] - x[3][1])
        return {1: (b[0] + d[1], b[1] - d[0]), 3: (b[0] - d[1], b[1] + d[0])}
    A = half([Q[0], Q[2], Q[4], Q[6]]); Bv = half([Q[1], Q[3], Q[5], Q[7]])
    h = f32c(np.sqrt(0.5)); o = {}
    for s in A:
        Ar, Ai = A[s]; br, bi = Bv[s]
        k = kp + 16 * s; km = 127 - kp - 16 * (s + 4)
        if s == 0:   Br, Bi, nBi = br, bi, None
        elif s == 1: Br, Bi, nBi = (br + bi) * h, (bi - br) * h, None
        elif s == 2: Br, Bi, nBi = bi, None, br
        else:        Br, Bi, nBi = (bi - br) * h, None, (br + bi) * h
        if 0 < k < NU:
            Re = Ar + Br
            Im = Ai + Bi if nBi is None else Ai - nBi
            o[k] = (Re, Im - Re, Re + Im)
        if 0 < km < NU:
            Re2 = Ar - Br
            if nBi is None:
                nIm2 = Bi - Ai
                o[km] = (Re2, nIm2 - Re2, Re2 + nIm2)
            else:
                pIm2 = nBi + Ai
                o[km] = (Re2, -(pIm2 + Re2), Re2 - pIm2)
    return o

def dft4c(x0, x1, y2, y3):
    c = (x1[0] + y3[0], x1[1] - y3[1]); d = (x1[0] - y3[0], x1[1] + y3[1])
    if x0 is None:
        assert y2 is None
        return [c, (d[1], -d[0]), (-c[0], -c[1]), (-d[1], d[0])]
    a = (x0[0] + y2[0], x0[1] - y2[1]); b = (x0[0] - y2[0], x0[1] + y2[1])
    return [(a[0] + c[0], a[1] + c[1]), (b[0] + d[1], b[1] - d[0]), (a[0] - c[0], a[1] - c[1]), (b[0] - d[1], b[1] + d[0])]
def dft8(x):
    A = dft4c(x[0], x[2], x[4], x[6]); Bv = dft4c(x[1], x[3], x[5], x[7])
    h = f32c(np.sqrt(0.5))
    b0, b1, b2, b3 = Bv
    t1 = ((b1[0] + b1[1]) * h, (b1[1] - b1[0]) * h)
    out = [None] * 8
    out[0] = (A[0][0] + b0[0], A[0][1] + b0[1]); out[4] = (A[0][0] - b0[0], A[0][1] - b0[1])
    out[1] = (A[1][0] + t1[0], A[1][1] + t1[1]); out[5] = (A[1][0] - t1[0], A[1][1] - t1[1])
    out[2] = (A[2][0] + b2[1], A[2][1] - b2[0]); out[6] = (A[2][0] - b2[1], A[2][1] + b2[0])
    u3 = (b3[1] - b3[0]) * h; v3 = (b3[0] + b3[1]) * h
    out[3] = (A[3][0] + u3, A[3][1] - v3); out[7] = (A[3][0] - u3, A[3][1] + v3)
    return out
def inv6(P):
    h = f32c(np.sqrt(0.5)); y = [None] * 6
    for par in range(2):
        R = []
        for k in range(2):
            x, z = P[k], P[3 - k]
            if par == 0: v = (x[0] + z[0], x[1] - z[1])
            else:
                v = (x[0] - z[0], x[1] + z[1]); v = cmul(v, -2 * np.pi * (k + 0.5) / 8)
            R.append(v)
        (r0, i0), (r1, i1) = R
        y[par] = r0 + r1
        y[par + 2] = ((r0 + i0) + (i1 - r1)) * h
        y[par + 4] = i0 - i1
    return y
def invB(Q, odd):
    P = []
    for k in range(4):
        x, z = Q[k], Q[7 - k]
        if not odd: P.append((x[0] + z[0], x[1] - z[1]))
        else: P.append(cmul((x[0] - z[0], x[1] + z[1]), -2 * np.pi * (k + 0.5) / 16))
    return inv6(P)


def make(B, T, D, K, UI=14, NI0=7, NI1=7, SP=2, scopes=True, TOKR=(0, 1, 2, 3), NP=6, NX0=2, WPL=4, NIL=3, NIH=7, LAG=0, TAIL=8, TAIL1=40, TH0=(0, 1), TH1=(0, 1), FOLD=True, TKB=4, TKA=4, FINE=True):
    M = T // 2; NJ = -(-M // L); MP = (NJ - 1) * L + N; NR = B * NJ
    f32 = jnp.float32; bf16 = jnp.bfloat16; i32 = jnp.int32
    JP = NJ // NP; TP = JP * 2 * L; TL = T - (NP - 1) * TP
    UM0 = NU // NI0; WP0 = -(-32 // NI0)
    UM1 = NU // NI1; NSP = NI1 * SP; JM = NR - 8 * NSP
    assert 0 < JM <= NR and JM % 4 == 0
    JH = NR - JM
    def odd4(n): return n + 4 if n % 8 == 0 else n
    SA = odd4(2 * JM); SB = odd4(2 * JH)
    def pieces_of(J0, J1, sem0):
        out = []; J = J0
        while J < J1:
            n = min(UI, J1 - J, NJ - J % NJ); out.append((J, n, sem0 + len(out))); J += n
        return out
    PCA = pieces_of(0, JM, 0); PCC = pieces_of(JM, NR, len(PCA))
    assert NJ % NP == 0 and NJ % UI == 0 and NU % NI0 == 0 and NU % UM1 == 0
    def bc(x, t): return pltpu.bitcast(x, t)
    def pack(a, b): return pltpu.pack_elementwise([a, b], packed_dtype=bf16)
    scope = jax.named_scope if scopes else (lambda n: contextlib.nullcontext())
    R3 = 2 * 192 * 128
    R2 = 2 * 128 * SW
    assert B * NJ * L <= R2
    H2 = D // 2
    PS = 2048 + 128; PV = 4096
    OC = B * NJ * L
    assert OC + 2 * NK * SB <= R2
    FG = JM // JP
    assert JM % JP == 0 and NR % JM == 0 and NX0 < FG

    def kernel(x_hbm, w_hbm, c_hbm, out_hbm,
               cbuf, wbuf, wbuf1, Xf, r2, r3, Ya, Yb, vbuf, Ps, zbuf, csem, xsem, wsem, osem, w1sem, vsem):
        x16 = Yb.bitcast(bf16); wb16 = wbuf.bitcast(bf16); w116 = wbuf1.bitcast(bf16); o16 = r2.bitcast(bf16); v16 = vbuf.bitcast(bf16)
        mk = pltpu.make_async_copy
        mo = pl.multiple_of
        ccopy = mk(c_hbm, cbuf, csem.at[0])
        def wcopy(i, h):
            return mk(w_hbm.at[i, pl.ds(mo(h * H2, 8), H2), pl.ds(0, 128)],
                      wb16.at[0, pl.ds(mo(i * (2 * SI) + h * H2, 8), H2), :], wsem.at[h])
        def wcopyg(i):
            return mk(w_hbm.at[i, :, pl.ds(D, 128)], wb16.at[1, pl.ds(mo(i * (2 * SI), 8), D), :], wsem.at[2])
        def w1copy(qh):
            e2 = qh // 2; h = qh % 2
            return mk(w_hbm.at[:, pl.ds(mo(h * H2, 8), H2), pl.ds(mo((1 + 2 * e2) * 128, 128), 128)], w116.at[qh], w1sem.at[qh])
        def xcopy(b, dt, p):
            n = TP if p < NP - 1 else TL
            return xcp(b, dt, p, n)
        def xcp(b, dt, p, n):
            row0 = mo(b * (2 * MP) + 64 + p * TP, 8)
            return mk(x_hbm.at[b, pl.ds(mo(p * TP, 8), n), pl.ds(dt * 128, 128)], x16.at[dt, pl.ds(row0, n), :], xsem.at[b * 2 + dt, p])
        def xstart(g):
            b, p = divmod(g, NP)
            for dt in range(2): xcopy(b, dt, p).start()
        def ocp(pc, c):
            J, nb, si = pc; b, j = divmod(J, NJ)
            t0 = j * 2 * L; n = min(T, (j + nb) * 2 * L) - t0
            return mk(o16.at[pl.ds(J * 2 * L, n), :], out_hbm.at[b, pl.ds(t0, n), pl.ds(mo(c * 128, 128), 128)], osem.at[si])

        @pl.loop(0, K)
        def _(i): wcopy(i, 0).start()
        ccopy.start()
        @pl.loop(0, K)
        def _(i): wcopy(i, 1).start()
        @pl.loop(0, K)
        def _(i): wcopyg(i).start()
        for g in range(NX0): xstart(g)
        zero = jnp.zeros
        for s in range(B * 2):
            Yb[s % 2, pl.ds((s // 2) * MP, 32), :] = zero((32, 128), i32)
            Yb[s % 2, pl.ds((s // 2) * MP + 32 + M, MP - 32 - M), :] = zero((MP - 32 - M, 128), i32)
        for e2 in range(2):
            wbuf[e2, pl.ds(K * SI, (32 - K) * SI), :] = zero(((32 - K) * SI, 128), i32)
            Ya[e2, pl.ds(NU * SA, 2 * JM), :] = zero((2 * JM, 128), i32)
        zbuf[...] = zero((8, 128), i32)
        ccopy.wait()
        GWr = lambda: bc(cbuf[0:256, :], bf16)
        FAr = lambda: bc(cbuf[256:320, :], bf16)
        IAr = lambda: bc(cbuf[320:368, :], bf16)
        SGN = lambda: bc(cbuf[368:376, :], f32)

        def wgroup(e2, g):
            tiles = []
            for qp in range(4):
                q0 = g * 8 + qp * 2
                t = jnp.concatenate([wbuf[e2, pl.ds(q0, 32, stride=SI), :], wbuf[e2, pl.ds(q0 + 1, 32, stride=SI), :]], axis=0)
                tiles.append(bc(t, bf16))
            o = jnp.dot(GWr(), jnp.concatenate(tiles, axis=1), preferred_element_type=f32)
            sg = SGN()
            for qp in range(4):
                col = qp * 128
                for qs in range(2):
                    q = g * 8 + qp * 2 + qs
                    for kg in range(8):
                        base = qs * 256 + kg * 32
                        r0 = o[base:base + 8, col:col + 128]; r1 = o[base + 8:base + 16, col:col + 128]
                        i0 = o[base + 16:base + 24, col:col + 128]; i1 = o[base + 24:base + 32, col:col + 128]
                        j0, j1 = (i0 * sg, i1 * sg) if kg == 0 else (i0, i1)
                        row = e2 * 128 * SW + q * SW + kg * 8
                        r2[pl.ds(row, 8), :] = pack(r0, r1)
                        r2[pl.ds(row + 64, 8), :] = pack(i0 - r0, i1 - r1)
                        r2[pl.ds(row + 128, 8), :] = pack(r0 + j0, r1 + j1)
        def phaseW0():
            for e2 in range(2):
                for h in range(2):
                    if e2 == 0:
                        if h == 1:
                            for g in range(NX0, B * NP):
                                xstart(g)
                                if g % FG == FG - 1 and g // FG < 2: w1copy(g // FG).start()
                            for qh in range(2, 4): w1copy(qh).start()
                        for i in range(K): wcopy(i, h).wait()
                    elif h == 0:
                        for i in range(K): wcopyg(i).wait()
                    for u in range(8): wgroup(e2, h * 8 + u)

        def fblock(b, j):
            tiles = []
            for dt in range(2):
                X = Yb[dt, pl.ds(b * MP + j * L, N), :]
                top = X[0:64]; bot = X[64:128]
                E = (top & 0xFFFF) | (bot << 16)
                O = lax.shift_right_logical(top, 16) | (bot & jnp.int32(-65536))
                tiles += [bc(E, bf16), bc(O, bf16)]
            Y = jnp.dot(FAr(), jnp.concatenate(tiles, axis=1), preferred_element_type=f32)
            J = b * NJ + j
            for dt in range(2):
                Ye = Y[:, dt * 256:dt * 256 + 128]; Yo = Y[:, dt * 256 + 128:dt * 256 + 256]
                Xf[dt, pl.ds(J * SX, 64), :] = pack(Ye[:64] + Ye[64:], Yo[:64] + Yo[64:])
                Xf[dt, pl.ds(J * SX + 64, 64), :] = pack(Ye[:64], Yo[:64])
                Xf[dt, pl.ds(J * SX + 128, 64), :] = pack(Ye[64:], Yo[64:])
        def phaseF(it):
            for u in range(FG):
                g = it * FG + u; b = g // NP; p = g % NP
                @pl.when(p < NP - 1)
                def _():
                    for dt in range(2): xcp(b, dt, p, TP).wait()
                @pl.when(p == NP - 1)
                def _():
                    for dt in range(2): xcp(b, dt, p, TL).wait()
            for u in range(FG):
                g = it * FG + u; b = g // NP; p = g % NP
                for v in range(JP): fblock(b, p * JP + v)

        def wvpu_pieces(wp, slot):
            e2 = wp // 16; qv = wp % 16
            pb = slot * PS
            out_row = lambda v, k: e2 * (192 * 128) + (v * 64 + k) * 128 + qv * 8
            pieces = []
            def p1(r, pos):
                def run(tok):
                    taps = [r + 8 * a for a in range(4)]
                    words = [wbuf1[e2 * 2 + qv // 8, i, pl.ds(mo((qv % 8) * 8, 8), 8), :] | tok if i < K else None for i in taps]
                    u = [None if wd is None else pltpu.unpack_elementwise(wd, index=pos, packed_dtype=bf16, unpacked_dtype=f32) for wd in words]
                    Pv = pass1(u)
                    for kp in range(8):
                        z = Pv[kp] if r == 0 else cmul(Pv[kp], -2 * np.pi * (kp + 0.5) / N * r)
                        base = pb + ((kp * 2 + pos) * 8 + r) * 16
                        Ps[pl.ds(base, 8), :] = z[0]
                        Ps[pl.ds(base + 8, 8), :] = z[1]
                    s = (u[0] + u[2]) + (u[1] + u[3] if u[3] is not None else u[1])
                    Ps[pl.ds(pb + 2048 + (pos * 8 + r) * 8, 8), :] = s
                return run
            def p2(kp, odd):
                def run(tok):
                    outs = []
                    for pos in range(2):
                        base = pb + ((kp * 2 + pos) * 8) * 16
                        Q = [[Ps[pl.ds(base + r * 16, 8), :], Ps[pl.ds(base + r * 16 + 8, 8), :]] for r in range(8)]
                        for r in TOKR:
                            for h in TH0: Q[r][h] = bc(bc(Q[r][h], i32) | tok, f32)
                        outs.append(p2half(Q, odd, kp))
                    for k in outs[0]:
                        for v in range(3):
                            r3[pl.ds(out_row(v, k), 8), :] = pack(outs[0][k][v], outs[1][k][v])
                return run
            def p3(tok):
                res = []
                for pos in range(2):
                    s = [Ps[pl.ds(pb + 2048 + (pos * 8 + r) * 8, 8), :] for r in range(8)]
                    s[0] = bc(bc(s[0], i32) | tok, f32); s[1] = bc(bc(s[1], i32) | tok, f32)
                    we = (s[0] + s[2]) + (s[4] + s[6]); wo = (s[1] + s[3]) + (s[5] + s[7])
                    res.append((we, wo - we, we - wo))
                for v in range(3):
                    r3[pl.ds(out_row(v, 0), 8), :] = pack(res[0][v], res[1][v])
            for r in range(8):
                for pos in range(2): pieces.append((p1(r, pos), 60 if r == 0 else 108))
            pieces.append((p3, 30))
            for kp in range(8):
                for odd in range(2): pieces.append((p2(kp, odd), 108 if odd else 92))
            return pieces

        def mbin(k, c, J0=0, J1=NR):
            def lhs(v): return jnp.concatenate([bc(Xf[dt, pl.ds(J0 * SX + v * 64 + k, J1 - J0, stride=SX), :], bf16) for dt in range(2)], axis=1)
            if c == 0:
                def rhs(v): return jnp.concatenate([bc(r2[pl.ds(e2 * 128 * SW + v * 64 + k, 128, stride=SW), :], bf16) for e2 in range(2)], axis=1)
            else:
                def rhs(v): return jnp.concatenate([bc(r3[pl.ds(mo(e2 * (192 * 128) + (v * 64 + k) * 128, 8), 128), :], bf16) for e2 in range(2)], axis=1)
            k1 = jnp.dot(lhs(0), rhs(0), preferred_element_type=f32)
            k2 = jnp.dot(lhs(1), rhs(1), preferred_element_type=f32)
            k3 = jnp.dot(lhs(2), rhs(2), preferred_element_type=f32)
            Yr = k1 - k3; Yi = k1 + k2
            nlo = 2 * (min(J1, JM) - J0) if J0 < JM else 0
            for e2 in range(2):
                cs = slice(e2 * 128, e2 * 128 + 128)
                if nlo: Ya[e2, pl.ds(k * SA, nlo), :] = pack(Yr[:nlo, cs], Yi[:nlo, cs])
                if J1 > JM:
                    hi = pack(Yr[nlo:, cs], Yi[nlo:, cs])
                    if c == 0: Yb[e2, pl.ds(k * SB, 2 * JH), :] = hi
                    else: r2[pl.ds(OC + (e2 * NK + k) * SB, 2 * JH), :] = hi
            return [k1, k2, k3]
        def place(ps, ks, lo, hi, nbins, zm):
            RG = ks[0].shape[0] // 8; G = 3 * RG
            tot = float(sum(wt for _, wt in ps)); acc = 0.0
            for p, wt in ps:
                pos = min(int(round(lo + acc / tot * (hi - lo))), nbins * G - 1)
                acc += wt
                d, g = divmod(pos, RG)
                p(bc(ks[d][g * 8:g * 8 + 8, 0:128], i32) & zm)
        def phaseM0(J0, J1, wp0, nwp, NI0):
            UM0 = NU // NI0
            G = 3 * (2 * (J1 - J0) // 8)
            @pl.loop(0, NI0)
            def _(kk):
                for q in range(4):
                    if wp0 <= 8 * q < wp0 + nwp * NI0:
                        @pl.when(kk == (8 * q - wp0) // nwp)
                        def _(): w1copy(q).wait()
                zm = zbuf[...]
                ks = []
                for u in range(UM0): ks += mbin(kk * UM0 + u, 0, J0, J1)
                ps = []
                for u in range(nwp):
                    ps += wvpu_pieces(jnp.minimum(wp0 + kk * nwp + u, 31), u % 2)
                place(ps, ks, LAG, UM0 * G - TAIL, UM0, zm)
        SO = L + 4
        NLAST = T - (NJ - 1) * 2 * L
        def vcopy(sp, u, n):
            J = JM + 8 * sp + u
            b = (J >= NJ).astype(i32)
            return mk(v16.at[pl.ds(mo(2 * (8 * sp + u) * SO, 8), n), :],
                      out_hbm.at[b, pl.ds(mo((J - b * NJ) * 2 * L, 8), n), pl.ds(0, 128)], vsem.at[0])
        def vop(sp, op):
            for u in range(8):
                if u == 7 or (JM <= NJ - 1 and u == (NJ - 1 - JM) % 8):
                    J = JM + 8 * sp + u
                    last = jnp.logical_or(J == NJ - 1, J == NR - 1)
                    @pl.when(last)
                    def _(): getattr(vcopy(sp, u, NLAST), op)()
                    @pl.when(jnp.logical_not(last))
                    def _(): getattr(vcopy(sp, u, 2 * L), op)()
                else:
                    getattr(vcopy(sp, u, 2 * L), op)()
        def ivpu_pieces(sp, slot):
            J0 = JM + 8 * sp
            pb = slot * PV
            pieces = []
            def qrow(pos, kp, rho): return pb + ((pos * 8 + kp) * 8 + rho) * 16
            def pA(kp, pos):
                p, e2 = divmod(pos, 2)
                def run(tok):
                    x = []
                    for s_ in range(8):
                        k = kp + 16 * s_
                        kk = k if k < 64 else 127 - k
                        if kk == 0 or kk >= NU:
                            x.append(None); continue
                        wd = Yb[e2, pl.ds(kk * SB + 16 * sp + p, 8, stride=2), :]
                        if s_ < TKA: wd = wd | tok
                        re = pltpu.unpack_elementwise(wd, index=0, packed_dtype=bf16, unpacked_dtype=f32)
                        im = pltpu.unpack_elementwise(wd, index=1, packed_dtype=bf16, unpacked_dtype=f32)
                        x.append((re, im))
                    Z = dft8(x)
                    for rho in range(8):
                        sc = 0.5 if (FOLD and e2 == 1) else 1.0
                        if rho == 0: z = Z[0] if sc == 1.0 else (Z[0][0] * sc, Z[0][1] * sc)
                        else: z = cmul(Z[rho], -2 * np.pi * (kp + 0.5) / N * rho, sc)
                        Ps[pl.ds(qrow(pos, kp, rho), 8), :] = z[0]
                        Ps[pl.ds(qrow(pos, kp, rho) + 8, 8), :] = z[1]
                return run
            held = {}
            def pBpos(rho, odd, p, e2, tok):
                pos = p * 2 + e2
                Q = [[Ps[pl.ds(qrow(pos, kp, rho), 8), :], Ps[pl.ds(qrow(pos, kp, rho) + 8, 8), :]] for kp in range(8)]
                for kp in range(TKB):
                    for h in TH1: Q[kp][h] = bc(bc(Q[kp][h], i32) | tok, f32)
                y = invB(Q, odd)
                wd = Yb[e2, pl.ds(16 * sp + p, 8, stride=2), :]
                sp_v = pltpu.unpack_elementwise(wd, index=rho % 2, packed_dtype=bf16, unpacked_dtype=f32)
                if FOLD and e2 == 1: sp_v = sp_v * 0.5
                h = [v + sp_v for v in y]
                if e2 == 0:
                    held['f'] = [jnp.tanh(v) for v in h]
                    return
                o = [f * (jnp.tanh(g if FOLD else g * 0.5) * 0.5 + 0.5) for f, g in zip(held['f'], h)]
                if p == 0: held[0] = o
                else:
                    for ap in range(6):
                        r = rho + 8 * (2 * ap + odd)
                        vbuf[pl.ds(8 * sp * SO + r, 8, stride=SO), :] = pack(held[0][ap], o[ap])
            def pB(rho, odd, p, e2s):
                def run(tok):
                    for e2 in e2s: pBpos(rho, odd, p, e2, tok)
                return run
            for kp in range(8):
                for pos in range(4): pieces.append((pA(kp, pos), 118))
            for rho in range(8):
                for odd in range(2):
                    for p in range(2):
                        if FINE:
                            pieces.append((pB(rho, odd, p, (0,)), (86 if odd else 62)))
                            pieces.append((pB(rho, odd, p, (1,)), (105 if odd else 81) + 6 * p))
                        else: pieces.append((pB(rho, odd, p, (0, 1)), (190 if odd else 143) + 6 * p))
            return pieces
        def phaseM1():
            RG = 2 * NR // 8; G = 3 * RG
            @pl.loop(0, NI1)
            def _(kk):
                zm = zbuf[...]
                ks = []
                for u in range(UM1): ks += mbin(kk * UM1 + u, 1)
                ps = []
                for u in range(SP): ps += ivpu_pieces(kk * SP + u, u % 2)
                place(ps, ks, LAG, UM1 * G - TAIL1, UM1, zm)
                for u in range(SP): vop(kk * SP + u, 'start')

        def iblock(J):
            tiles = []
            for p in range(2):
                for e2 in range(2):
                    if J < JM: t = Ya[e2, pl.ds(2 * J + p, 64, stride=SA), :]
                    else: t = r2[pl.ds(OC + e2 * NK * SB + 2 * (J - JM) + p, 64, stride=SB), :]
                    tiles.append(bc(t, bf16))
            h = jnp.dot(IAr(), jnp.concatenate(tiles, axis=1), preferred_element_type=f32)
            oe = jnp.tanh(h[:, 0:128]) * (jnp.tanh(h[:, 128:256] * 0.5) * 0.5 + 0.5)
            oo = jnp.tanh(h[:, 256:384]) * (jnp.tanh(h[:, 384:512] * 0.5) * 0.5 + 0.5)
            r2[pl.ds(J * L, L), :] = pack(oe, oo)
        def phaseI(pcs, c):
            for pc in pcs:
                for J in range(pc[0], pc[0] + pc[1]): iblock(J)
                ocp(pc, c).start()

        with scope('W'): phaseW0()
        @pl.loop(0, NR // JM)
        def _(it):
            with scope('F'): phaseF(it)
            @pl.when(it == 0)
            def _():
                with scope('M0l'): phaseM0(0, JM, 0, WPL, NIL)
        @pl.loop(0, 2)
        def _(c):
            @pl.when(c == 0)
            def _():
                with scope('M0h'): phaseM0(JM, NR, WPL * NIL, -(-(32 - WPL * NIL) // NIH), NIH)
            @pl.when(c == 1)
            def _():
                for e2 in range(2):
                    r2[pl.ds(OC + (e2 * NK + NU) * SB, 2 * JH), :] = zero((2 * JH, 128), i32)
                with scope('M1'): phaseM1()
                for pc in PCA: ocp(pc, 0).wait()
            with scope('IA'): phaseI(PCA, c)
        with scope('IC'): phaseI(PCC, 1)
        with scope('end'):
            @pl.loop(0, NSP)
            def _(h): vop(h, 'wait')
            for pc in PCA + PCC: ocp(pc, 1).wait()

    cst = consts(K)
    def f(x, w):
        return pl.pallas_call(kernel,
            out_shape=jax.ShapeDtypeStruct((B, T, D), bf16),
            in_specs=[pl.BlockSpec(memory_space=pl.ANY)] * 3,
            out_specs=pl.BlockSpec(memory_space=pl.ANY),
            scratch_shapes=[pltpu.VMEM(cst.shape, i32), pltpu.VMEM((2, 32 * SI, 128), i32), pltpu.VMEM((4, K, 64, 128), i32),
                            pltpu.VMEM((2, NR * SX, 128), i32), pltpu.VMEM((R2, 128), i32), pltpu.VMEM((R3, 128), i32),
                            pltpu.VMEM((2, NK * SA, 128), i32), pltpu.VMEM((2, max(NK * SB, B * MP), 128), i32), pltpu.VMEM((max(JH, 8) * (L + 4), 128), i32), pltpu.VMEM((2 * PV, 128), f32), pltpu.VMEM((8, 128), i32),
                            pltpu.SemaphoreType.DMA((1,)), pltpu.SemaphoreType.DMA((B * 2, NP)), pltpu.SemaphoreType.DMA((3,)),
                            pltpu.SemaphoreType.DMA((len(PCA) + len(PCC),)), pltpu.SemaphoreType.DMA((4,)),
                            pltpu.SemaphoreType.DMA((1,))],
            compiler_params=pltpu.CompilerParams(vmem_limit_bytes=127 * 1024 * 1024),
        )(x, w, jnp.asarray(cst))
    return f


@jax.jit
def pallas_standalone__autoregressive_conv_wavernn__speech_kernel(x: jax.Array, w: jax.Array):
    B, T, D = x.shape
    K = w.shape[0]
    return make(B, T, D, K, scopes=False)(x, w)
```
